```python
import os as _os
_os.environ.setdefault('JAX_PLATFORMS', 'cpu')
import jax
import jax.numpy as jnp

def _softmax(x, axis=-1):
    return jax.nn.softmax(x, axis=axis)

def _gelu(x):
    return jax.nn.gelu(x, approximate=True)

def _silu(x):
    return jax.nn.silu(x)

def _sigmoid(x):
    return jax.nn.sigmoid(x)

def _layernorm(x, axis=-1, eps=1e-05):
    m = jnp.mean(x, axis=axis, keepdims=True)
    v = jnp.var(x, axis=axis, keepdims=True)
    return (x - m) / jnp.sqrt(v + eps)

def _scatter_add(tgt, idx, src, axis=0):
    return tgt.at[idx].add(src)

def _segment_sum(src, seg, n):
    return jax.ops.segment_sum(src, seg, n)

class _Rng:

    def __init__(self, key):
        self._k = key

    def _next(self):
        self._k, sub = jax.random.split(self._k)
        return sub

    def normal(self, shape):
        return jax.random.normal(self._next(), shape, dtype=jnp.bfloat16)

    def randint(self, lo, hi, shape):
        return jax.random.randint(self._next(), shape, lo, hi, dtype=jnp.int32)

    def uniform(self, shape, lo=0.0, hi=1.0):
        return jax.random.uniform(self._next(), shape, jnp.bfloat16, lo, hi)

    def permutation(self, n):
        return jax.random.permutation(self._next(), n)
kernel_name = 'adaLN_cond__sliding_block__mixer_channel_mlp__prompt'

def setup_inputs():
    _rng = _Rng(jax.random.key(int.from_bytes(__import__("os").urandom(4), "little")))
    _w = lambda a: (lambda t: t.astype(jnp.bfloat16) if jnp.issubdtype(t.dtype, jnp.floating) else t)(jnp.asarray(a))

    def _A_setup():
        B, S, D = (1, 2048, 640)
        return {'x': _w((lambda *s: _rng.normal(s) * 0.05)(B, S, D)), 'wqkv': _w((lambda *s: _rng.normal(s) * 0.05)(D, 3 * D)), 'wo': _w((lambda *s: _rng.normal(s) * 0.05)(D, D))}
    _A_in = _A_setup()

    def _B_setup():
        B, S, D, F = (1, 2048, 640, 1728)
        return {'x': _w((lambda *s: _rng.normal(s) * 0.05)(B, S, D)), 'w1': _w((lambda *s: _rng.normal(s) * 0.8)(D, F) * D ** (-0.5)), 'b1': _w((lambda *s: _rng.normal(s) * 0.8)(F)), 'w2': _w((lambda *s: _rng.normal(s) * 0.8)(F, D) * F ** (-0.5)), 'b2': _w((lambda *s: _rng.normal(s) * 0.4)(D))}
    _B_in = _B_setup()
    return {'A_x': _A_in['x'], 'A_wqkv': _A_in['wqkv'], 'A_wo': _A_in['wo'], 'B_x': _B_in['x'], 'B_w1': _B_in['w1'], 'B_b1': _B_in['b1'], 'B_w2': _B_in['w2'], 'B_b2': _B_in['b2'], 'c': _w((lambda *s: _rng.normal(s) * 0.05)(1, 640) * 8.0), 'w_mod': _w((lambda *s: _rng.normal(s) * 0.05)(640, 6 * 640) * 640 ** (-0.5) * 8.0)}

def reference(A_x, A_wqkv, A_wo, B_x, B_w1, B_b1, B_w2, B_b2, c, w_mod):

    def _A_ref(x, wqkv, wo):
        B, S, D = x.shape
        H = 32
        Dh = D // H
        W = 256
        qkv = (lambda x, *d: x.transpose(*d))((x @ wqkv).reshape(B, S, 3, H, Dh), 2, 0, 3, 1, 4)
        q, k, v = (qkv[0], qkv[1], qkv[2])
        scores = jnp.einsum('bhqd,bhkd->bhqk', q, k) * Dh ** (-0.5)
        idx = jnp.arange(S)
        mask = (idx[:, None] - idx[None, :] >= 0) & (idx[:, None] - idx[None, :] < W)
        scores = jnp.where(mask[None, None], scores, -1000000000.0)
        p = _softmax(scores, axis=-1)
        o = jnp.einsum('bhqk,bhkd->bhqd', p, v)
        return (lambda x, *d: x.transpose(*d))(o, 0, 2, 1, 3).reshape(B, S, D) @ wo

    def _B_ref(x, w1, b1, w2, b2):
        y = _layernorm(x, axis=-1)
        h = _gelu(jnp.einsum('bsd,df->bsf', y, w1) + b1)
        return jnp.einsum('bsf,fd->bsd', h, w2) + b2
    x = A_x
    mod = (_silu(c) @ w_mod).reshape(c.shape[0], 6, 1, -1)
    sa, ca, ga, sb, cb, gb = (mod[:, 0].copy(), mod[:, 1].copy(), mod[:, 2].copy(), mod[:, 3].copy(), mod[:, 4].copy(), mod[:, 5].copy())
    h = _layernorm(x, axis=-1) * (1 + ca) + sa
    x = x + ga * _A_ref(h, A_wqkv, A_wo)
    h = _layernorm(x, axis=-1) * (1 + cb) + sb
    x = x + gb * _B_ref(h, B_w1, B_b1, B_w2, B_b2)
    return x
```

```python
import functools
import jax
import jax.numpy as jnp
from jax import lax
import jax.experimental.pallas as pl
import jax.experimental.pallas.tpu as pltpu

S = 2048
D = 640
H = 32
DH = 20
W = 256
F = 1728
TQ = 256
NB = S // TQ
NSUB = TQ // 128
EPS = 1e-5
F32 = jnp.float32
BF16 = jnp.bfloat16
U32 = jnp.uint32
LOG2E = 1.4426950408889634
QSCALE = (DH ** -0.5) * LOG2E
NT = (((1,), (1,)), ((), ()))


def _ln(x):
    m = jnp.mean(x, axis=-1, keepdims=True)
    xc = x - m
    v = jnp.mean(xc * xc, axis=-1, keepdims=True)
    return xc * lax.rsqrt(v + EPS)


def _gelu(x):
    c1 = 0.7978845608028654
    c2 = c1 * 0.044715
    u = x * (c1 + c2 * (x * x))
    return (0.5 * x) * (1.0 + jnp.tanh(u))


def _pack(x):
    return pltpu.bitcast(x.astype(BF16), U32)


def _unpack(x):
    return pltpu.bitcast(x, BF16)


def _pair_tile(j):
    lo, hi = 40 * j, 40 * j + 40
    if lo // 128 == (hi - 1) // 128:
        t = lo // 128
        return t, lo - 128 * t
    t = (lo - 64) // 128
    assert t == (hi - 1 - 64) // 128
    return 5 + t, lo - 64 - 128 * t


def _kernel(x_ref, wqkv_ref, wo_ref, w1t_ref, b1_ref, w2_ref, b2_ref, c_ref, wmod_ref, o_ref,
            mod_sc, k_sc, vt_sc, ot_sc):
    i = pl.program_id(0)

    @pl.when(i == 0)
    def _():
        c = c_ref[...].astype(F32)
        sc = (c * jax.nn.sigmoid(c)).astype(BF16)
        sc = jnp.broadcast_to(sc, (16, D))
        mod_sc[...] = jnp.dot(sc, wmod_ref[...], preferred_element_type=F32)[0:8]
        vt_sc[0:2] = jnp.zeros((2, H * 16, 128), U32)

    def mod(n):
        return mod_sc[0:1, n * D:(n + 1) * D]

    row0h = pl.multiple_of(i * (TQ // 2), TQ // 2)
    ones = jnp.ones((8, 128), F32)
    xs, qs = [], []
    for bb in range(NSUB):
        x = x_ref[128 * bb:128 * bb + 128, :].astype(F32)
        xs.append(x)
        h = (_ln(x) * (1.0 + mod(1)) + mod(0)).astype(BF16)
        qkv = jnp.dot(h, wqkv_ref[...], preferred_element_type=F32)
        q32 = _pack(qkv[:, 0:D] * QSCALE)
        kf = qkv[:, D:2 * D]
        k32 = _pack(kf)
        qs.append(jnp.concatenate([q32, q32[:, 64:576]], axis=1))
        k_sc[pl.ds(row0h + (W // 2 + 64 * bb), 64), :] = jnp.concatenate([k32, k32[:, 64:576]], axis=1)
        if bb == 0:
            pad0 = pl.multiple_of(jnp.where(i == 0, 0, (S + W) // 2), W // 2)
            k0 = _pack(jnp.broadcast_to(kf[0:1], (16, D)))
            k0 = jnp.concatenate([k0, k0[:, 64:576]], axis=1)
            k_sc[pl.ds(pad0, W // 2), :] = jnp.concatenate([k0] * (W // 16), axis=0)
        vt = qkv[:, 2 * D:3 * D].T
        for hd in range(H):
            st = 8 * ((20 * hd) // 8)
            vt_sc[2 + i * NSUB + bb, 16 * hd:16 * hd + 16, :] = _pack(
                jnp.concatenate([vt[st:st + 24], ones], axis=0))

    lane = lax.broadcasted_iota(jnp.int32, (32, 128), 1)
    row = lax.broadcasted_iota(jnp.int32, (32, 128), 0)
    ql = lane & 63
    tri32 = (jnp.where(2 * row <= ql, jnp.uint32(0xFFFF), jnp.uint32(0))
             | jnp.where(2 * row + 1 <= ql, jnp.uint32(0xFFFF0000), jnp.uint32(0)))
    lane_lo = lane < 64
    tri = lax.broadcasted_iota(jnp.int32, (64, 128), 0) <= (lax.broadcasted_iota(jnp.int32, (64, 128), 1) & 63)
    sub8 = lax.broadcasted_iota(jnp.int32, (8, 128), 0) < 4
    z32 = jnp.zeros((32, 128), U32)

    def qk_unit(base, t, qm):
        parts = []
        for u in range(4):
            parts.append(k_sc[pl.ds(base + 8 * u, 8), 128 * t:128 * t + 128])
            parts.append(k_sc[pl.ds(base + 128 + 8 * u, 8), 128 * t:128 * t + 128])
        parts.append(k_sc[pl.ds(base + 32, 96), 128 * t:128 * t + 128])
        kk = _unpack(jnp.concatenate(parts, axis=0))
        s = lax.dot_general(kk, _unpack(qm), NT, preferred_element_type=F32)
        merged = jnp.concatenate(
            [jnp.where(tri[16 * u:16 * u + 16], s[32 * u + 16:32 * u + 32], s[32 * u:32 * u + 16])
             for u in range(4)], axis=0)
        sm = jnp.concatenate([merged, s[128:320]], axis=0)
        m = jnp.max(sm, axis=0, keepdims=True)
        return sm, m

    def stage_a(bb, j):
        t, off = _pair_tile(j)
        qq = qs[bb][:, 128 * t:128 * t + 128]
        ma = (lane >= off) & (lane < off + 20)
        mb = (lane >= off + 20) & (lane < off + 40)
        qlo, qhi = qq[0:32], qq[32:64]
        qm_lo = jnp.concatenate([jnp.where(ma, qlo, z32), jnp.where(mb, qlo, z32)], axis=0)
        qm_hi = jnp.concatenate([jnp.where(mb, qhi, z32), jnp.where(ma, qhi, z32)], axis=0)
        base = pl.multiple_of(row0h + 64 * bb, 64)
        return qk_unit(base, t, qm_lo), qk_unit(base + 32, t, qm_hi)

    def stage_b(bb, j, lo, hi):
        def probs(sm, m):
            p = _pack(jnp.exp2(sm - m))
            last = p[0:32] & tri32
            first = p[0:32] ^ last
            return [first, p[32:64], p[64:96], p[96:128], last]
        c_lo = probs(*lo) + [z32]
        c_hi = [z32] + probs(*hi)
        p_a = jnp.concatenate([jnp.where(lane_lo, a, b) for a, b in zip(c_lo, c_hi)], axis=0)
        p_b = jnp.concatenate([jnp.where(lane_lo, b, a) for a, b in zip(c_lo, c_hi)], axis=0)
        tb = i * NSUB + bb
        outs = []
        for hd, p in ((2 * j, p_a), (2 * j + 1, p_b)):
            vth = jnp.concatenate([vt_sc[tb + u, 16 * hd:16 * hd + 16, :] for u in range(3)], axis=1)
            o = jnp.dot(_unpack(vth), _unpack(p), preferred_element_type=F32)
            r = 1.0 / o[24:32]
            outs.append(o[0:24] * jnp.concatenate([r, r, r], axis=0))
        oa, ob = outs
        ob = pltpu.roll(ob, 64, 1)
        pair = jnp.concatenate([oa[0:16], jnp.where(sub8, oa[16:24], ob[0:8]), ob[8:24]], axis=0)
        ot_sc[bb, 40 * j:40 * j + 40, :] = pair

    groups = [(bb, g) for bb in range(NSUB) for g in range(H // 4)]
    pend = None
    for n in range(len(groups) + 1):
        cur = None
        if n < len(groups):
            bb, g = groups[n]
            cur = [(bb, j, stage_a(bb, j)) for j in (2 * g, 2 * g + 1)]
        if pend is not None:
            for bb, j, (lo, hi) in pend:
                stage_b(bb, j, lo, hi)
        pend = cur

    x1s, ys = [], []
    for bb in range(NSUB):
        o = ot_sc[bb].T.astype(BF16)
        attn = jnp.dot(o, wo_ref[...], preferred_element_type=F32)
        x1 = xs[bb] + mod(2) * attn
        h2 = _ln(x1) * (1.0 + mod(4)) + mod(3)
        x1s.append(x1)
        ys.append(_ln(h2).astype(BF16))
    gs = []
    for bb in range(NSUB):
        h1 = lax.dot_general(ys[bb], w1t_ref[...], NT, preferred_element_type=F32) + b1_ref[...].astype(F32)
        gs.append(_gelu(h1).astype(BF16))
    for bb in range(NSUB):
        mlp = jnp.dot(gs[bb], w2_ref[...], preferred_element_type=F32) + b2_ref[...].astype(F32)
        o_ref[128 * bb:128 * bb + 128, :] = (x1s[bb] + mod(5) * mlp).astype(o_ref.dtype)


@jax.jit
def pallas_adaLN_cond__sliding_block__mixer_channel_mlp__prompt_kernel(
    A_x, A_wqkv, A_wo, B_x, B_w1, B_b1, B_w2, B_b2, c, w_mod):
    del B_x
    x = A_x.reshape(S, D)
    const = lambda shape: pl.BlockSpec(shape, lambda i: (0,) * len(shape), pipeline_mode=pl.Buffered(1))
    out = pl.pallas_call(
        _kernel,
        grid=(NB,),
        in_specs=[
            pl.BlockSpec((TQ, D), lambda i: (i, 0)),
            const((D, 3 * D)), const((D, D)), const((F, D)), const((1, F)), const((F, D)), const((1, D)),
            const((1, D)), const((D, 6 * D)),
        ],
        out_specs=pl.BlockSpec((TQ, D), lambda i: (i, 0)),
        out_shape=jax.ShapeDtypeStruct((S, D), A_x.dtype),
        scratch_shapes=[
            pltpu.VMEM((8, 6 * D), F32),
            pltpu.VMEM(((S + 2 * W) // 2, 9 * 128), U32),
            pltpu.VMEM((S // 128 + 2, H * 16, 128), U32),
            pltpu.VMEM((NSUB, D, 128), F32),
        ],
        compiler_params=pltpu.CompilerParams(
            dimension_semantics=("arbitrary",), vmem_limit_bytes=100 * 1024 * 1024),
        name="fused_block",
    )(x, A_wqkv, A_wo, B_w1.T, B_b1.reshape(1, F), B_w2, B_b2.reshape(1, D), c, w_mod)
    return out.reshape(1, S, D)
```

```python
import functools
import jax
import jax.numpy as jnp
from jax import lax
import jax.experimental.pallas as pl
import jax.experimental.pallas.tpu as pltpu

S = 2048
D = 640
H = 32
DH = 20
W = 256
F = 1728
TQ = 256
NB = S // TQ
NSUB = TQ // 128
NG = H // 4
NP = 8
TORDER = (1, 0, 2)
CORDER = (3, 2, 1, 0)
STEP = 3
LN1_CH = 4
LN2_CH = 1
QSPLIT = 1024
P1_AT = 11
EPS = 1e-5
F32 = jnp.float32
BF16 = jnp.bfloat16
U32 = jnp.uint32
LOG2E = 1.4426950408889634
QSCALE = (DH ** -0.5) * LOG2E
NT = (((1,), (1,)), ((), ()))


def _rowsum(x, zero=None):
    t = x[:, 0:128]
    for j in range(1, D // 128):
        t = t + x[:, 128 * j:128 * j + 128]
    if zero is not None:
        t = t + jnp.concatenate([zero] * (x.shape[0] // 8), axis=0)
    return jnp.sum(t, axis=-1, keepdims=True)


def _ln(x, zero=None):
    xc = x - _rowsum(x, zero) * (1.0 / D)
    v = _rowsum(xc * xc) * (1.0 / D)
    return xc * lax.rsqrt(v + EPS)


def _gelu(x):
    c1 = 0.7978845608028654
    c2 = c1 * 0.044715
    u = x * (c1 + c2 * (x * x))
    return (0.5 * x) * (1.0 + jnp.tanh(u))


def _dot_cols(a, w_ref, lo, hi, parts=1, nt=False):
    def dot(x, c0, c1):
        if nt:
            return lax.dot_general(x, w_ref[c0:c1, :], NT, preferred_element_type=F32)
        return jnp.dot(x, w_ref[:, c0:c1], preferred_element_type=F32)
    if parts == 1:
        return dot(a, lo, hi)
    mid = (hi - 1) // 128 * 128
    r = 128 // parts
    return jnp.concatenate([
        dot(a, lo, mid),
        jnp.concatenate([dot(a[r * e:r * e + r], mid, hi) for e in range(parts)], axis=0)], axis=1)


def _xor_rows(x):
    hl = (lax.broadcasted_iota(jnp.int32, (32, D), 1) // DH) & 3
    m0, m1 = (hl & 1) == 0, (hl & 2) == 0
    r = [x[32 * s:32 * s + 32] for s in range(4)]
    t = [jnp.where(m0, r[s], r[s ^ 1]) for s in range(4)]
    return jnp.concatenate([jnp.where(m1, t[s], t[s ^ 2]) for s in range(4)], axis=0)


def _unpack(x):
    return pltpu.bitcast(x, BF16)


def _group_tile(g):
    lo, hi = 80 * g, 80 * g + 80
    if lo // 128 == (hi - 1) // 128:
        t = lo // 128
        return t, lo - 128 * t
    t = (lo - 64) // 128
    assert t == (hi - 1 - 64) // 128
    return 5 + t, lo - 64 - 128 * t


def _kernel(x_hbm, wqkv_hbm, wo_hbm, w1t_hbm, b1_hbm, w2_hbm, b2_hbm, c_hbm, wmod_hbm, o_ref,
            x_sc, wqkv_sc, wo_sc, w1t_sc, b1_sc, w2_sc, b2_sc, c_sc, wmod_sc, sems,
            mod_sc, h_sc, q_sc, k_sc, vt_sc, p_sc0, p_sc1, *rest):
    ot_sc, s_sc = rest[:NSUB], rest[NSUB:]
    i = pl.program_id(0)
    z1 = lax.shift_right_logical(i, 20)
    z2 = lax.shift_right_logical(i, 21)
    q32 = q_sc.bitcast(U32)
    k32 = k_sc.bitcast(U32)
    vt32 = vt_sc.bitcast(U32)

    def cols(a, b):
        return (wmod_hbm.at[:, a * D:b * D], wmod_sc.at[:, a * D:b * D])

    def wcols(a):
        return (wqkv_hbm.at[:, a * D:(a + 1) * D], wqkv_sc.at[:, a * D:(a + 1) * D])

    pairs = {
        "c": (c_hbm, c_sc),
        "x0": (x_hbm.at[0:TQ], x_sc.at[0:TQ]),
        "modA": cols(0, 2),
        "wq": wcols(0),
        "wk": wcols(1),
        "wv": wcols(2),
        "modB": cols(2, 5),
        "wo": (wo_hbm, wo_sc),
        "b1": (b1_hbm, b1_sc),
        "b2": (b2_hbm, b2_sc),
        "w1": (w1t_hbm, w1t_sc),
        "w2": (w2_hbm, w2_sc),
        "modC": cols(5, 6),
        "x1": (x_hbm.at[TQ:2 * TQ], x_sc.at[TQ:2 * TQ]),
        "x2": (x_hbm.at[2 * TQ:3 * TQ], x_sc.at[2 * TQ:3 * TQ]),
        "x3": (x_hbm.at[3 * TQ:S], x_sc.at[3 * TQ:S]),
    }
    copies = {name: pltpu.make_async_copy(src, dst, sems.at[n])
              for n, (name, (src, dst)) in enumerate(pairs.items())}

    def wait(*names):
        for name in names:
            copies[name].wait()

    def mod(n):
        return mod_sc[0:1, n * D:(n + 1) * D]

    def compute_mod(a, b):
        c = c_sc[...].astype(F32)
        sc = jnp.broadcast_to((c * jax.nn.sigmoid(c)).astype(BF16), (16, D))
        mod_sc[:, a * D:b * D] = jnp.dot(sc, wmod_sc[:, a * D:b * D], preferred_element_type=F32)[0:8]

    def store_tiles(ref, ref32, r0, n, val):
        for t in range(5):
            ref[t, pl.ds(r0, n), :] = val[:, 128 * t:128 * t + 128].astype(BF16)
        r0h = r0 // 2 if isinstance(r0, int) else pl.multiple_of(r0 // 2, 8)
        full = jnp.concatenate([ref32[t, pl.ds(r0h, n // 2), :] for t in range(5)], axis=1)
        for t in range(4):
            ref32[5 + t, pl.ds(r0h, n // 2), :] = full[:, 64 + 128 * t:192 + 128 * t]

    def body(first):
        p_sc = p_sc0 if first else p_sc1
        p32 = p_sc.bitcast(U32)
        if first:
            blk, row0, row0h = 0, 0, 0
        else:
            blk = i
            row0 = pl.multiple_of(i * TQ, TQ)
            row0h = pl.multiple_of(i * (TQ // 2), TQ // 2)

        lane = lax.broadcasted_iota(jnp.int32, (16, 128), 1)
        row = lax.broadcasted_iota(jnp.int32, (16, 128), 0)
        ql = lane & 31
        tri32 = (jnp.where(2 * row <= ql, jnp.uint32(0xFFFF), jnp.uint32(0))
                 | jnp.where(2 * row + 1 <= ql, jnp.uint32(0xFFFF0000), jnp.uint32(0)))
        tri = [row <= ql, row + 16 <= ql]
        bit0 = (lane & 32) == 0
        bit1 = lane < 64
        bit0_24 = (lax.broadcasted_iota(jnp.int32, (24, 128), 1) & 32) == 0
        sub8 = lax.broadcasted_iota(jnp.int32, (8, 128), 0) < 4
        z16 = jnp.zeros((16, 128), U32)
        always = lax.broadcasted_iota(jnp.int32, (8, 128), 1) >= z1
        qcode = ((lax.broadcasted_iota(jnp.int32, (40, 128), 1) >> 5)
                 ^ (lax.broadcasted_iota(jnp.int32, (40, 128), 0) // (DH // 2)))

        def chained(fn, nch):
            r = 128 // nch
            outs, zero = [], None
            for e in range(nch):
                res = fn(slice(r * e, r * e + r), zero)
                outs.append(res)
                zero = jnp.where(always, 0.0, res[-1][0:8, 0:128])
            return [jnp.concatenate(parts, axis=0) for parts in zip(*outs)]

        def ln1(r0):
            x = x_sc[pl.ds(r0, 128), :].astype(F32)
            return chained(lambda rs, zero: (_ln(x[rs], zero) * (1.0 + mod(1)) + mod(0),), LN1_CH)[0].astype(BF16)

        hs, qkvs = {}, {0: [], 1: []}

        def put_q(bb, qf):
            q_sc[bb] = _xor_rows(qf * QSCALE).T.astype(BF16)

        def put_k(bb, kf):
            kr = row0 + (W + 128 * bb)
            store_tiles(k_sc, k32, kr if first else pl.multiple_of(kr, 128), 128, kf)
            if first and bb == 0:
                store_tiles(k_sc, k32, 0, W, jnp.broadcast_to(kf[0:1], (W, D)))

        def put_v(bb, vf):
            vt = vf.T
            ones = jnp.ones((8, 128), F32)
            for hd in range(H):
                st = 8 * ((20 * hd) // 8)
                vt_sc[2 + blk * NSUB + bb, 32 * hd:32 * hd + 32, :] = (
                    jnp.concatenate([vt[st:st + 24], ones], axis=0).astype(BF16))

        def qkv_stage(bb, lo, hi, parts):
            if bb not in hs:
                hs[bb] = h_sc[...] if bb == 0 else ln1(row0 + 128 * bb)
            qkvs[bb].append(_dot_cols(hs[bb], wqkv_sc, lo, hi, parts))
            if hi < 3 * D:
                return
            qkv = jnp.concatenate(qkvs[bb], axis=1)
            put_q(bb, qkv[:, 0:D])
            put_k(bb, qkv[:, D:2 * D])
            put_v(bb, qkv[:, 2 * D:3 * D])

        def sel(m, a, b):
            if a is None and b is None:
                return None
            return jnp.where(m, z16 if a is None else a, z16 if b is None else b)

        maxes = {}

        def stage_a(n):
            bb, g = divmod(n, NG)
            t, off = _group_tile(g)
            zq = q32[bb, 40 * g:40 * g + 40, :]
            base = row0h + 64 * bb
            base = base if first else pl.multiple_of(base, 64)
            ms = []
            for u in range(4):
                parts = [jnp.zeros((off // 2, 128), U32), jnp.where(qcode == u, zq, jnp.zeros_like(zq)),
                         jnp.zeros((24 - off // 2, 128), U32)]
                qm = jnp.concatenate([p for p in parts if p.shape[0]], axis=0)
                kb = base + 16 * u
                kk = jnp.concatenate([
                    k32[t, pl.ds(kb, 8), :], k32[t, pl.ds(kb + 128, 8), :],
                    k32[t, pl.ds(kb + 8, 8), :], k32[t, pl.ds(kb + 136, 8), :],
                    k32[t, pl.ds(kb + 16, 112), :]], axis=0)
                s = jnp.dot(_unpack(kk), _unpack(qm), preferred_element_type=F32)
                sm = jnp.concatenate([jnp.where(tri[0], s[16:32], s[0:16]),
                                      jnp.where(tri[1], s[48:64], s[32:48]), s[64:288]], axis=0)
                s_sc[(4 * n + u) % NP][z1] = sm
                acc = [sm[0:8], sm[8:16]]
                for r in range(2, 32):
                    acc[r % 2] = jnp.maximum(acc[r % 2], sm[8 * r:8 * r + 8])
                ms.append(jnp.max(jnp.maximum(acc[0], acc[1]), axis=0, keepdims=True))
            maxes[n] = ms

        def stage_b(n):
            bb, g = divmod(n, NG)
            items = []
            for t in TORDER:
                for c in CORDER:
                    for u in range(4):
                        k = (4 * t + c - u) % 8
                        if 0 <= 4 * t + c - u <= 8 and (u, k) not in items:
                            items.append((u, k))
            ms = [jnp.broadcast_to(m, (8, 128)) for m in maxes.pop(n)]
            pk = {}
            prev = None
            for e in range(0, 32, STEP):
                for u, k in items[e:e + STEP]:
                    slot = (4 * n + u) % NP
                    m = ms[u] if prev is None else jnp.where(always, ms[u], prev)
                    p = jnp.exp2(s_sc[slot][z2, 32 * k:32 * k + 32, :] - jnp.concatenate([m] * 4, axis=0))
                    p_sc[u, 32 * k:32 * k + 32, :] = p.astype(BF16)
                    pk[u, k] = p32[u, 16 * k:16 * k + 16, :]
                prev = p[0:8]
            units = []
            for u in range(4):
                last = pk[u, 0] & tri32
                chunks = [pk[u, 0] ^ last] + [pk[u, k] for k in range(1, 8)] + [last]
                units.append([None] * u + chunks + [None] * (3 - u))
            ph = [[], [], [], []]
            for c in range(12):
                u0, u1, u2, u3 = (units[u][c] for u in range(4))
                a0, a1, a2, a3 = sel(bit0, u0, u1), sel(bit0, u1, u0), sel(bit0, u2, u3), sel(bit0, u3, u2)
                ph[0].append(sel(bit1, a0, a2))
                ph[1].append(sel(bit1, a1, a3))
                ph[2].append(sel(bit1, a2, a0))
                ph[3].append(sel(bit1, a3, a1))
            tb = blk * NSUB + bb
            part = {}
            for t in TORDER:
                for hh in range(4):
                    hd = 4 * g + hh
                    part[hh, t] = jnp.dot(_unpack(vt32[tb + t, 16 * hd:16 * hd + 16, :]),
                                          _unpack(jnp.concatenate(ph[hh][4 * t:4 * t + 4], axis=0)),
                                          preferred_element_type=F32)
            outs = []
            for hh in range(4):
                d0, d1, d2 = (part[hh, t] for t in TORDER)
                o = d0[0:24] + d1[0:24] + d2[0:24]
                den = d0[24:32] + d1[24:32] + d2[24:32]
                r = pl.reciprocal(den, approx=True)
                r = r * (2.0 - den * r)
                o = o * jnp.concatenate([r, r, r], axis=0)
                if hh == 1:
                    o = jnp.where(bit0_24, pltpu.roll(o, 96, 1), pltpu.roll(o, 32, 1))
                elif hh == 2:
                    o = pltpu.roll(o, 64, 1)
                elif hh == 3:
                    o = jnp.where(bit0_24, pltpu.roll(o, 32, 1), pltpu.roll(o, 96, 1))
                outs.append(o)
            for e in range(2):
                oa, ob = outs[2 * e], outs[2 * e + 1]
                pair = jnp.concatenate([oa[0:16], jnp.where(sub8, oa[16:24], ob[0:8]), ob[8:24]], axis=0)
                ot_sc[bb][z1, 80 * g + 40 * e:80 * g + 40 * e + 40, :] = pair

        x1s, ys, gs = {}, {}, {}

        def wo_stage(bb, parts):
            o = ot_sc[bb][z2].T.astype(BF16)
            attn = _dot_cols(o, wo_sc, 0, D, parts)
            x1 = x_sc[pl.ds(row0 + 128 * bb, 128), :].astype(F32) + mod(2) * attn
            x1s[bb] = x1
            ys[bb] = chained(lambda rs, zero: (_ln(_ln(x1[rs], zero) * (1.0 + mod(4)) + mod(3)),),
                             LN2_CH)[0].astype(BF16)

        def w1_stage(bb, parts):
            b1 = b1_sc[...].astype(F32).reshape(1, F)
            gs[bb] = _gelu(_dot_cols(ys[bb], w1t_sc, 0, F, parts, nt=True) + b1).astype(BF16)

        def w2_stage(bb, lo, hi, parts):
            b2 = b2_sc[...].astype(F32).reshape(1, D)
            mlp = _dot_cols(gs[bb], w2_sc, lo, hi, parts) + b2[:, lo:hi]
            o_ref[128 * bb:128 * bb + 128, lo:hi] = (
                x1s[bb][:, lo:hi] + mod(5)[:, lo:hi] * mlp).astype(o_ref.dtype)

        def attention(lo, hi):
            stage_a(lo)
            for n in range(lo, hi - 1):
                stage_a(n + 1)
                stage_b(n)

        last = NSUB * NG - 1
        if first:
            for cp in copies.values():
                cp.start()
            vt_sc[0:2] = jnp.zeros((2, H * 32, 128), BF16)
            wait("c", "x0")
            xn = _ln(x_sc[0:TQ, :].astype(F32))
            wait("modA")
            compute_mod(0, 2)
            h = (xn * (1.0 + mod(1)) + mod(0)).astype(BF16)
            h = [h[128 * bb:128 * bb + 128] for bb in range(NSUB)]
            wait("wq")
            qf = [_dot_cols(h[bb], wqkv_sc, 0, D, 2) for bb in range(NSUB)]
            wait("wk")
            kf = [_dot_cols(h[bb], wqkv_sc, D, 2 * D, 2) for bb in range(NSUB)]
            wait("wv")
            vf = [_dot_cols(h[bb], wqkv_sc, 2 * D, 3 * D, 2) for bb in range(NSUB)]
            for bb in range(NSUB):
                put_q(bb, qf[bb])
                put_k(bb, kf[bb])
                put_v(bb, vf[bb])
            attention(0, P1_AT)
            stage_a(P1_AT)
            wait("modB", "wo")
            compute_mod(2, 5)
            stage_b(P1_AT - 1)
            wo_stage(0, 4)
            for n in range(P1_AT, last - 1):
                stage_a(n + 1)
                stage_b(n)
            stage_a(last)
            wait("b1", "b2", "w1")
            b1 = b1_sc[...].astype(F32).reshape(1, F)
            b2 = b2_sc[...].astype(F32).reshape(1, D)
            g0 = [_gelu(_dot_cols(ys[0], w1t_sc, 0, 256, 2, nt=True) + b1[:, 0:256])]
            stage_b(last - 1)
            g0.append(_gelu(_dot_cols(ys[0], w1t_sc, 256, 512, 2, nt=True) + b1[:, 256:512]))
            stage_b(last)
            g0.append(_gelu(_dot_cols(ys[0], w1t_sc, 512, 1024, nt=True) + b1[:, 512:1024]))
            wo_stage(1, 4)
            g0.append(_gelu(_dot_cols(ys[0], w1t_sc, 1024, F, nt=True) + b1[:, 1024:F]))
            gs[0] = jnp.concatenate(g0, axis=1).astype(BF16)
            h1 = _dot_cols(ys[1], w1t_sc, 0, F, nt=True) + b1
            g1 = _gelu(h1[:, 0:1280])
            wait("w2")
            gs[1] = jnp.concatenate([g1, _gelu(h1[:, 1280:F])], axis=1).astype(BF16)
            m0 = _dot_cols(gs[0], w2_sc, 0, D, 2) + b2
            wait("modC", "x1")
            compute_mod(5, 6)
            o_ref[0:128, :] = (x1s[0] + mod(5) * m0).astype(o_ref.dtype)
            h_sc[...] = ln1(TQ)
            w2_stage(1, 0, D, 1)
        else:
            qkv_stage(0, 0, 3 * D, 4)
            attention(0, NG)
            qkv_stage(1, 0, 512, 1)
            stage_b(NG - 1)
            qkv_stage(1, 512, QSPLIT, 1)
            wo_stage(0, 1)
            qkv_stage(1, QSPLIT, 3 * D, 1)
            w1_stage(0, 2)
            attention(NG, 2 * NG)
            w2_stage(0, 0, 256, 1)
            stage_b(last)
            w2_stage(0, 256, 384, 1)
            wo_stage(1, 4)
            w2_stage(0, 384, D, 1)
            w1_stage(1, 1)
            h_sc[...] = ln1(pl.multiple_of(jnp.minimum(i + 1, NB - 1) * TQ, TQ))
            w2_stage(1, 0, D, 1)

    pl.when(i == 1)(functools.partial(wait, "x2"))
    pl.when(i == 2)(functools.partial(wait, "x3"))
    pl.when(i == 0)(functools.partial(body, True))
    pl.when(i > 0)(functools.partial(body, False))


@jax.jit
def pallas_adaLN_cond__sliding_block__mixer_channel_mlp__prompt_kernel(
    A_x, A_wqkv, A_wo, B_x, B_w1, B_b1, B_w2, B_b2, c, w_mod):
    del B_x
    x = A_x.reshape(S, D)
    out = pl.pallas_call(
        _kernel,
        grid=(NB,),
        in_specs=[pl.BlockSpec(memory_space=pl.ANY)] * 9,
        out_specs=pl.BlockSpec((TQ, D), lambda i: (i, 0)),
        out_shape=jax.ShapeDtypeStruct((S, D), A_x.dtype),
        scratch_shapes=[
            pltpu.VMEM((S, D), BF16),
            pltpu.VMEM((D, 3 * D), BF16),
            pltpu.VMEM((D, D), BF16),
            pltpu.VMEM((F, D), BF16),
            pltpu.VMEM((F,), BF16),
            pltpu.VMEM((F, D), BF16),
            pltpu.VMEM((D,), BF16),
            pltpu.VMEM((1, D), BF16),
            pltpu.VMEM((D, 6 * D), BF16),
            pltpu.SemaphoreType.DMA((16,)),
            pltpu.VMEM((8, 6 * D), F32),
            pltpu.VMEM((128, D), BF16),
            pltpu.VMEM((NSUB, D, 128), BF16),
            pltpu.VMEM((9, S + W, 128), BF16),
            pltpu.VMEM((S // 128 + 2, H * 32, 128), BF16),
            pltpu.VMEM((4, 256, 128), BF16),
            pltpu.VMEM((4, 256, 128), BF16),
        ] + [pltpu.VMEM((1, D, 128), F32)] * NSUB + [pltpu.VMEM((1, 256, 128), F32)] * NP,
        compiler_params=pltpu.CompilerParams(
            dimension_semantics=("arbitrary",), vmem_limit_bytes=100 * 1024 * 1024),
        name="fused_block",
    )(x, A_wqkv, A_wo, B_w1.T, B_b1, B_w2, B_b2, c, w_mod)
    return out.reshape(1, S, D)
```

```python
import functools

import jax
import jax.numpy as jnp
from jax import lax
import jax.experimental.pallas as pl
import jax.experimental.pallas.tpu as pltpu

S = 2048
D = 640
H = 32
DH = 20
F = 1728
NFIRST = 4
NSUB = 2
NSTEP = 1 + (S // 128 - NFIRST) // NSUB
NG = H // 4
NP = 8
C1, C2 = 384, 1024
QE = 3 * D - 128
EPS = 1e-5
NEG = -1e30
F32 = jnp.float32
BF16 = jnp.bfloat16
U32 = jnp.uint32
QSCALE = (DH ** -0.5) * 1.4426950408889634
NT = (((1,), (1,)), ((), ()))


def _rowsum(x, zero=None):
    t = x[:, 0:128]
    for j in range(1, D // 128):
        t = t + x[:, 128 * j:128 * j + 128]
    if zero is not None:
        t = t + jnp.concatenate([zero] * (x.shape[0] // 8), axis=0)
    return jnp.sum(t, axis=-1, keepdims=True)


def _ln(x, zero=None):
    xc = x - _rowsum(x, zero) * (1.0 / D)
    v = _rowsum(xc * xc) * (1.0 / D)
    return xc * lax.rsqrt(v + EPS)


def _gelu(x):
    c1 = 0.7978845608028654
    c2 = c1 * 0.044715
    u = x * (c1 + c2 * (x * x))
    return (0.5 * x) * (1.0 + jnp.tanh(u))


def _dot_cols(a, w_ref, lo, hi, parts=1, nt=False):
    def dot(x, c0, c1):
        x = x.astype(BF16)
        if nt:
            return lax.dot_general(x, w_ref[c0:c1, :], NT, preferred_element_type=F32)
        return jnp.dot(x, w_ref[:, c0:c1], preferred_element_type=F32)
    if parts == 1:
        return dot(a, lo, hi)
    mid = (hi - 1) // 128 * 128
    r = a.shape[0] // parts
    head = [dot(a, lo, mid)] if lo < mid else []
    return jnp.concatenate(
        head + [jnp.concatenate([dot(a[r * e:r * e + r], mid, hi) for e in range(parts)], axis=0)], axis=1)


def _xor_rows(x):
    hl = (lax.broadcasted_iota(jnp.int32, (32, D), 1) // DH) & 3
    m0, m1 = (hl & 1) == 0, (hl & 2) == 0
    r = [x[32 * s:32 * s + 32] for s in range(4)]
    t = [jnp.where(m0, r[s], r[s ^ 1]) for s in range(4)]
    return jnp.concatenate([jnp.where(m1, t[s], t[s ^ 2]) for s in range(4)], axis=0)


def _unpack(x):
    return pltpu.bitcast(x, BF16)


def _group_tile(g):
    lo, hi = 80 * g, 80 * g + 80
    if lo // 128 == (hi - 1) // 128:
        t = lo // 128
        return t, lo - 128 * t
    t = (lo - 64) // 128
    assert t == (hi - 1 - 64) // 128
    return 5 + t, lo - 64 - 128 * t


def _kernel(x_hbm, wqkv_hbm, wo_hbm, w1t_hbm, b1_hbm, w2_hbm, b2_hbm, c_hbm, wmod_hbm, o_hbm,
            x_sc, wqkv_sc, wo_sc, w1t_sc, b1_sc, w2_sc, b2_sc, c_sc, wmod_sc, sems, o_sc, osem,
            mod_sc, h_sc, q_sc, k_sc, vt_sc, p_sc0, p_sc1, *rest):
    ot_sc, s_sc = rest[:NFIRST], rest[NFIRST:]
    i = pl.program_id(0)
    z1 = lax.shift_right_logical(i, 20)
    z2 = lax.shift_right_logical(i, 21)
    q32 = q_sc.bitcast(U32)
    k32 = k_sc.bitcast(U32)
    vt32 = vt_sc.bitcast(U32)

    def cols(src, dst, a, b):
        return (src.at[:, a:b], dst.at[:, a:b])

    def rows(a, b):
        return (x_hbm.at[a:b], x_sc.at[a:b])

    pairs = {
        "c": (c_hbm, c_sc),
        "x0": rows(0, 384),
        "ca": cols(wmod_hbm, wmod_sc, D, 2 * D),
        "wa": cols(wqkv_hbm, wqkv_sc, 0, C1),
        "wb": cols(wqkv_hbm, wqkv_sc, C1, C2),
        "wc": cols(wqkv_hbm, wqkv_sc, C2, 3 * D),
        "sa": cols(wmod_hbm, wmod_sc, 0, D),
        "x1": rows(384, 640),
        "modB": cols(wmod_hbm, wmod_sc, 2 * D, 5 * D),
        "wo": (wo_hbm, wo_sc),
        "b1": (b1_hbm, b1_sc),
        "b2": (b2_hbm, b2_sc),
        "w1": (w1t_hbm, w1t_sc),
        "w2": (w2_hbm, w2_sc),
        "modC": cols(wmod_hbm, wmod_sc, 5 * D, 6 * D),
        "x2": rows(640, S),
    }
    copies = {name: pltpu.make_async_copy(src, dst, sems.at[n])
              for n, (name, (src, dst)) in enumerate(pairs.items())}

    def wait(*names):
        for name in names:
            copies[name].wait()

    def mod(n):
        return mod_sc[0:1, n * D:(n + 1) * D]

    def compute_mod(a, b):
        c = c_sc[...].astype(F32)
        sc = jnp.broadcast_to((c * jax.nn.sigmoid(c)).astype(BF16), (16, D))
        mod_sc[:, a * D:b * D] = jnp.dot(sc, wmod_sc[:, a * D:b * D], preferred_element_type=F32)[0:8]

    def body(first):
        p_sc = p_sc0 if first else p_sc1
        p32 = p_sc.bitcast(U32)
        blk0 = 0 if first else NFIRST + (i - 1) * NSUB

        def at(bb, scale, off=0, align=8):
            v = (blk0 + bb) * scale + off
            return v if first else pl.multiple_of(v, align)

        def rows_of(bb):
            return pl.ds(at(bb, 128, align=128), 128)

        lane = lax.broadcasted_iota(jnp.int32, (16, 128), 1)
        row = lax.broadcasted_iota(jnp.int32, (16, 128), 0)
        ql = lane & 31
        tri = [row <= ql, row + 16 <= ql]
        tri32 = (jnp.where(2 * row <= ql, jnp.uint32(0xFFFF), jnp.uint32(0))
                 | jnp.where(2 * row + 1 <= ql, jnp.uint32(0xFFFF0000), jnp.uint32(0)))
        bit0 = (lane & 32) == 0
        bit1 = lane < 64
        bit0_24 = (lax.broadcasted_iota(jnp.int32, (24, 128), 1) & 32) == 0
        sub8 = lax.broadcasted_iota(jnp.int32, (8, 128), 0) < 4
        z16 = jnp.zeros((16, 128), U32)
        always = lax.broadcasted_iota(jnp.int32, (8, 128), 1) >= z1
        qcode = ((lax.broadcasted_iota(jnp.int32, (40, 128), 1) >> 5)
                 ^ (lax.broadcasted_iota(jnp.int32, (40, 128), 0) // (DH // 2)))

        def chained(fn, x, nch):
            r = x.shape[0] // nch
            outs, zero = [], None
            for e in range(nch):
                outs.append(fn(x[r * e:r * e + r], zero))
                zero = jnp.where(always, 0.0, outs[-1][0:8, 0:128])
            return jnp.concatenate(outs, axis=0)

        def ln1(rs, nch):
            return chained(lambda x, zero: _ln(x, zero) * (1.0 + mod(1)) + mod(0), x_sc[rs, :].astype(F32), nch)

        def put_qkv(bb, qkv):
            q_sc[bb] = _xor_rows(qkv[:, 0:D] * QSCALE).T.astype(BF16)
            for t in range(5):
                k_sc[t, rows_of(bb), :] = qkv[:, D + 128 * t:D + 128 * t + 128].astype(BF16)
            full = jnp.concatenate([k32[t, pl.ds(at(bb, 64), 64), :] for t in range(5)], axis=1)
            for t in range(4):
                k32[5 + t, pl.ds(at(bb, 64), 64), :] = full[:, 64 + 128 * t:192 + 128 * t]
            vt = qkv[:, 2 * D:3 * D].T
            ones = jnp.ones((8, 128), F32)
            for hd in range(H):
                st = 8 * ((DH * hd) // 8)
                vt_sc[blk0 + bb, 32 * hd:32 * hd + 32, :] = (
                    jnp.concatenate([vt[st:st + 24], ones], axis=0).astype(BF16))

        hs, qkvs = {}, {}

        def qkv_stage(bb, lo, hi):
            if bb not in hs:
                hs[bb] = h_sc[...] if bb == 0 else ln1(rows_of(bb), 4).astype(BF16)
                qkvs[bb] = {}
            qkvs[bb][lo] = _dot_cols(hs[bb], wqkv_sc, lo, hi)
            if sum(v.shape[1] for v in qkvs[bb].values()) == 3 * D:
                put_qkv(bb, jnp.concatenate([qkvs[bb][k] for k in sorted(qkvs[bb])], axis=1))

        def sel(m, a, b):
            if a is None and b is None:
                return None
            return jnp.where(m, z16 if a is None else a, z16 if b is None else b)

        jobs = {}

        def stage_a(n, parts, g):
            t, off = _group_tile(g)
            where, maxes = {}, {}
            used = [0] * 4
            for pi, (bb, cmin) in enumerate(parts):
                zq = q32[bb, 40 * g:40 * g + 40, :]
                for u in (range(4) if cmin == 0 else range(3, -1, -1)):
                    wts = [jnp.zeros((off // 2, 128), U32), jnp.where(qcode == u, zq, jnp.zeros_like(zq)),
                           jnp.zeros((24 - off // 2, 128), U32)]
                    qm = jnp.concatenate([w for w in wts if w.shape[0]], axis=0)
                    kmin = max(1, cmin - u)

                    def keys(r, n_):
                        return k32[t, pl.ds(at(bb, 64, 16 * u - 128 + r), n_), :]

                    mid = [keys(16 * kmin, 128 - 16 * kmin)] if kmin < 8 else []
                    if cmin == 0:
                        kk = jnp.concatenate([keys(0, 8), keys(128, 8), keys(8, 8), keys(136, 8)] + mid, axis=0)
                        s = jnp.dot(_unpack(kk), _unpack(qm), preferred_element_type=F32)
                        sm = [jnp.where(tri[0], s[16:32], s[0:16]), jnp.where(tri[1], s[48:64], s[32:48]), s[64:]]
                    else:
                        kk = jnp.concatenate([keys(128, 16)] + mid, axis=0)
                        s = jnp.dot(_unpack(kk), _unpack(qm), preferred_element_type=F32)
                        sm = [jnp.where(tri[0], s[0:16], NEG), jnp.where(tri[1], s[16:32], NEG)]
                        sm += [s[32:]] if mid else []
                    sm = jnp.concatenate(sm, axis=0)
                    nr = sm.shape[0]
                    v = u if pi == 0 else 3 - u
                    buf = s_sc[(4 * n + v) % NP]
                    buf[z1, used[v]:used[v] + nr, :] = sm
                    for j, k in enumerate([0] + list(range(kmin, 8))):
                        where[pi, u, k] = (buf, used[v] + 32 * j)
                    used[v] += nr
                    acc = [sm[0:8], sm[8:16]]
                    for r in range(2, nr // 8):
                        acc[r % 2] = jnp.maximum(acc[r % 2], sm[8 * r:8 * r + 8])
                    maxes[pi, u] = jnp.max(jnp.maximum(acc[0], acc[1]), axis=0, keepdims=True)
            jobs[n] = (parts, g, where, maxes)

        def stage_b(n, prev=None):
            parts, g, where, maxes = jobs.pop(n)
            tiles = [(pi, t) for pi, (_, cmin) in enumerate(parts) for t in (1, 0, 2) if 4 * t >= cmin]
            if len(parts) == 2:
                tiles = tiles[::-1]
            items = []
            for pi, t in tiles:
                for c in (3, 2, 1, 0):
                    for u in range(4):
                        it = (pi, u, (4 * t + c - u) % 8)
                        if 0 <= 4 * t + c - u <= 8 and it not in items:
                            items.append(it)
            assert sorted(items) == sorted(where)
            ms = {k: jnp.broadcast_to(m, (8, 128)) for k, m in maxes.items()}
            pk = {}
            step = len(parts) + 1
            for e in range(0, len(items), step):
                for pi, u, k in items[e:e + step]:
                    buf, r0 = where[pi, u, k]
                    m = ms[pi, u] if prev is None else jnp.where(always, ms[pi, u], prev)
                    p = jnp.exp2(buf[z2, r0:r0 + 32, :] - jnp.concatenate([m] * 4, axis=0))
                    p_sc[4 * pi + u, 32 * k:32 * k + 32, :] = p.astype(BF16)
                    pk[pi, u, k] = p32[4 * pi + u, 16 * k:16 * k + 16, :]
                    if (pi, u, k) == items[e]:
                        nxt = p[24:32]
                prev = nxt
            ph = {}
            for pi, (bb, cmin) in enumerate(parts):
                units = []
                for u in range(4):
                    if cmin == 0:
                        last = pk[pi, u, 0] & tri32
                        head = pk[pi, u, 0] ^ last
                    else:
                        last, head = pk[pi, u, 0], None
                    chunks = [head] + [pk.get((pi, u, k)) for k in range(1, 8)] + [last]
                    units.append([None] * u + chunks + [None] * (3 - u))
                for c in range(cmin, 12):
                    u0, u1, u2, u3 = (units[u][c] for u in range(4))
                    a0, a1, a2, a3 = sel(bit0, u0, u1), sel(bit0, u1, u0), sel(bit0, u2, u3), sel(bit0, u3, u2)
                    ph[pi, 0, c] = sel(bit1, a0, a2)
                    ph[pi, 1, c] = sel(bit1, a1, a3)
                    ph[pi, 2, c] = sel(bit1, a2, a0)
                    ph[pi, 3, c] = sel(bit1, a3, a1)
            part = {}
            for pi, t in tiles:
                for hh in range(4):
                    hd = 4 * g + hh
                    pt = jnp.concatenate([ph[pi, hh, c] for c in range(4 * t, 4 * t + 4)], axis=0)
                    part[pi, hh, t] = jnp.dot(_unpack(vt32[blk0 + parts[pi][0] - 2 + t, 16 * hd:16 * hd + 16, :]),
                                              _unpack(pt), preferred_element_type=F32)
            for pi, (bb, cmin) in enumerate(parts):
                outs = []
                for hh in range(4):
                    ds = [part[pi, hh, t] for pj, t in tiles if pj == pi]
                    o = functools.reduce(jnp.add, [d[0:24] for d in ds])
                    den = functools.reduce(jnp.add, [d[24:32] for d in ds])
                    r = pl.reciprocal(den, approx=True)
                    r = r * (2.0 - den * r)
                    o = o * jnp.concatenate([r, r, r], axis=0)
                    if hh == 1:
                        o = jnp.where(bit0_24, pltpu.roll(o, 96, 1), pltpu.roll(o, 32, 1))
                    elif hh == 2:
                        o = pltpu.roll(o, 64, 1)
                    elif hh == 3:
                        o = jnp.where(bit0_24, pltpu.roll(o, 32, 1), pltpu.roll(o, 96, 1))
                    outs.append(o)
                for e in range(2):
                    oa, ob = outs[2 * e], outs[2 * e + 1]
                    pair = jnp.concatenate([oa[0:16], jnp.where(sub8, oa[16:24], ob[0:8]), ob[8:24]], axis=0)
                    ot_sc[bb][z1, 80 * g + 40 * e:80 * g + 40 * e + 40, :] = pair

        def attention(*plist, hook=None, dep=None):
            todo = [(parts, g) for parts in plist for g in range(NG)]
            stage_a(0, *todo[0])
            for n in range(len(todo) - 1):
                stage_a(n + 1, *todo[n + 1])
                if hook is not None and n == len(todo) - 2:
                    hook()
                stage_b(n, dep if n == 0 else None)
            return functools.partial(stage_b, len(todo) - 1)

        x1s, ys, gs = {}, {}, {}

        def wo_stage(bb, halves=False, nch=1):
            o = ot_sc[bb][z2].T
            if halves:
                attn = jnp.concatenate([_dot_cols(o[64 * e:64 * e + 64], wo_sc, 0, D, 2) for e in range(2)], axis=0)
            else:
                attn = _dot_cols(o, wo_sc, 0, D, 4)
            x1s[bb] = x_sc[rows_of(bb), :].astype(F32) + mod(2) * attn
            ys[bb] = chained(lambda x, zero: _ln(_ln(x, zero) * (1.0 + mod(4)) + mod(3)), x1s[bb], nch)

        def w1_stage(bb, between=None, after=None):
            y = ys[bb]
            if between is None:
                head = _dot_cols(y, w1t_sc, 0, 768, nt=True)
            else:
                head = _dot_cols(y, w1t_sc, 0, 512, nt=True)
                between()
                head = jnp.concatenate([head, _dot_cols(y, w1t_sc, 512, 768, nt=True)], axis=1)
            fm = F - 64
            tail = (lax.dot_general(w1t_sc[fm:F, 0:512], y[:, 0:512].astype(BF16), NT, preferred_element_type=F32).T
                    + lax.dot_general(y[:, 512:D].astype(BF16), w1t_sc[fm:F, 512:D], NT, preferred_element_type=F32))
            h1 = jnp.concatenate([head, _dot_cols(y, w1t_sc, 768, fm, nt=True), tail], axis=1)
            h1 = h1 + b1_sc[...].astype(F32).reshape(1, F)
            if after is None:
                gs[bb] = _gelu(h1)
            else:
                g = [_gelu(h1[:, 0:fm - 256]), None, _gelu(h1[:, fm:F])]
                after()
                g[1] = _gelu(h1[:, fm - 256:fm])
                gs[bb] = jnp.concatenate(g, axis=1)

        def w2_stage(bb, lo=0, hi=D, parts=1):
            b2 = b2_sc[...].astype(F32).reshape(1, D)
            mlp = _dot_cols(gs[bb], w2_sc, lo, hi, parts) + b2[:, lo:hi]
            o_sc[rows_of(bb), lo:hi] = (x1s[bb][:, lo:hi] + mod(5)[:, lo:hi] * mlp).astype(o_sc.dtype)

        def flush(bb, lo=0, hi=D):
            pltpu.make_async_copy(o_sc.at[rows_of(bb), lo:hi], o_hbm.at[rows_of(bb), lo:hi], osem).start()

        if first:
            for cp in copies.values():
                cp.start()
            wait("c", "x0")
            xn = _ln(x_sc[0:384, :].astype(F32))
            wait("ca")
            compute_mod(1, 2)
            t = [xn[128 * bb:128 * bb + 128] * (1.0 + mod(1)) for bb in range(3)]
            res = [[], [], []]
            wait("wa")
            for bb in range(3):
                res[bb].append(_dot_cols(t[bb], wqkv_sc, 0, C1, 4 if bb == 2 else 1))
            wait("wb")
            for bb in range(3):
                res[bb].append(_dot_cols(t[bb], wqkv_sc, C1, C2, 4 if bb == 2 else 1))
            wait("wc")
            for bb in range(2):
                res[bb].append(_dot_cols(t[bb], wqkv_sc, C2, 3 * D, 2 if bb == 1 else 1))
            wait("sa", "x1")
            compute_mod(0, 1)
            res[2].append(_dot_cols(t[2], wqkv_sc, C2, 3 * D))
            h3 = ln1(rows_of(3), 1)
            sa = jnp.broadcast_to(mod(0), (16, D))
            r3 = jnp.concatenate(
                [_dot_cols(jnp.concatenate([h3, sa], axis=0), wqkv_sc, 0, QE),
                 jnp.concatenate([_dot_cols(h3, wqkv_sc, QE, 3 * D, 4), _dot_cols(sa, wqkv_sc, QE, 3 * D)], axis=0)],
                axis=1)
            for bb in range(4):
                put_qkv(bb, r3[0:128] if bb == 3 else jnp.concatenate(res[bb], axis=1) + r3[128:129])

            def mid_weights():
                wait("modB", "wo", "b1", "b2", "w1")
                compute_mod(2, 5)

            attention([(1, 4), (0, 8)], [(2, 0)], hook=mid_weights)()
            wo_stage(0)
            wo_stage(1)
            wo_stage(2)
            w1_stage(0)
            fin = attention([(3, 0)])
            w1_stage(1, fin, functools.partial(wait, "w2", "modC"))
            compute_mod(5, 6)
            wo_stage(3, halves=True)
            w2_stage(0)
            flush(0)
            w1_stage(2)
            w2_stage(1)
            flush(1)
            w1_stage(3)
            w2_stage(2)
            flush(2)
            h_sc[...] = ln1(rows_of(NFIRST), 8).astype(BF16)
            w2_stage(3, parts=2)
            flush(3)
        else:
            qkv_stage(0, 0, 3 * D)
            qkv_stage(1, QE, 3 * D)
            fin = attention([(0, 0)])
            qkv_stage(1, 0, 512)
            fin()
            qkv_stage(1, 512, 2 * D)
            wo_stage(0)
            qkv_stage(1, 2 * D, QE)
            y0 = functools.reduce(jnp.maximum, [ys[0][8 * r:8 * r + 8, 0:128] for r in range(16)])
            fin = attention([(1, 0)], dep=y0)
            w1_stage(0, fin)
            wo_stage(1, nch=4)
            w2_stage(0)
            w1_stage(1)
            flush(0)
            nxt = pl.multiple_of(jnp.minimum(blk0 + NSUB, S // 128 - 1) * 128, 128)
            h_sc[...] = ln1(pl.ds(nxt, 128), 8).astype(BF16)
            w2_stage(1, 0, 512)
            flush(1, 0, 512)
            w2_stage(1, 512, D, 2)
            flush(1, 512, D)

    pl.when(i == 1)(functools.partial(wait, "x2"))
    pl.when(i == 0)(functools.partial(body, True))
    pl.when(i > 0)(functools.partial(body, False))

    @pl.when(i == NSTEP - 1)
    def _():
        pltpu.make_async_copy(o_sc, o_hbm, osem).wait()


@jax.jit
def pallas_adaLN_cond__sliding_block__mixer_channel_mlp__prompt_kernel(
    A_x, A_wqkv, A_wo, B_x, B_w1, B_b1, B_w2, B_b2, c, w_mod):
    del B_x
    out = pl.pallas_call(
        _kernel,
        grid=(NSTEP,),
        in_specs=[pl.BlockSpec(memory_space=pl.ANY)] * 9,
        out_specs=pl.BlockSpec(memory_space=pl.ANY),
        out_shape=jax.ShapeDtypeStruct((S, D), A_x.dtype),
        scratch_shapes=[
            pltpu.VMEM((S, D), BF16),
            pltpu.VMEM((D, 3 * D), BF16),
            pltpu.VMEM((D, D), BF16),
            pltpu.VMEM((F, D), BF16),
            pltpu.VMEM((F,), BF16),
            pltpu.VMEM((F, D), BF16),
            pltpu.VMEM((D,), BF16),
            pltpu.VMEM((1, D), BF16),
            pltpu.VMEM((D, 6 * D), BF16),
            pltpu.SemaphoreType.DMA((16,)),
            pltpu.VMEM((S, D), BF16),
            pltpu.SemaphoreType.DMA(()),
            pltpu.VMEM((8, 6 * D), F32),
            pltpu.VMEM((128, D), BF16),
            pltpu.VMEM((NFIRST, D, 128), BF16),
            pltpu.VMEM((9, S, 128), BF16),
            pltpu.VMEM((S // 128, H * 32, 128), BF16),
            pltpu.VMEM((8, 256, 128), BF16),
            pltpu.VMEM((8, 256, 128), BF16),
        ] + [pltpu.VMEM((1, D, 128), F32)] * NFIRST
          + [pltpu.VMEM((1, 288, 128), F32)] * NP,
        compiler_params=pltpu.CompilerParams(
            dimension_semantics=("arbitrary",), vmem_limit_bytes=100 * 1024 * 1024,
            disable_bounds_checks=True, disable_semaphore_checks=True),
        name="fused_block",
    )(A_x.reshape(S, D), A_wqkv, A_wo, B_w1.T, B_b1, B_w2, B_b2, c, w_mod)
    return out.reshape(1, S, D)
```

```python
import functools

import jax
import jax.numpy as jnp
from jax import lax
import jax.experimental.pallas as pl
import jax.experimental.pallas.tpu as pltpu

S = 2048
D = 640
H = 32
DH = 20
F = 1728
NFIRST = 4
NSUB = 2
NSTEP = 1 + (S // 128 - NFIRST) // NSUB
NG = H // 4
NP = 8
C1, C2 = 384, 1024
QE = 3 * D - 128
EPS = 1e-5
NEG = -1e30
F32 = jnp.float32
BF16 = jnp.bfloat16
U32 = jnp.uint32
QSCALE = (DH ** -0.5) * 1.4426950408889634
NT = (((1,), (1,)), ((), ()))


def _rowsum(x, zero=None):
    t = x[:, 0:128]
    for j in range(1, D // 128):
        t = t + x[:, 128 * j:128 * j + 128]
    if zero is not None:
        t = t + jnp.concatenate([zero] * (x.shape[0] // 8), axis=0)
    return jnp.sum(t, axis=-1, keepdims=True)


def _ln(x, zero=None):
    xc = x - _rowsum(x, zero) * (1.0 / D)
    v = _rowsum(xc * xc) * (1.0 / D)
    return xc * lax.rsqrt(v + EPS)


def _gelu(x):
    c1 = 0.7978845608028654
    c2 = c1 * 0.044715
    u = x * (c1 + c2 * (x * x))
    return (0.5 * x) * (1.0 + jnp.tanh(u))


def _dot_cols(a, w_ref, lo, hi, parts=1, nt=False):
    def dot(x, c0, c1):
        x = x.astype(BF16)
        if nt:
            return lax.dot_general(x, w_ref[c0:c1, :], NT, preferred_element_type=F32)
        return jnp.dot(x, w_ref[:, c0:c1], preferred_element_type=F32)
    if parts == 1:
        return dot(a, lo, hi)
    mid = (hi - 1) // 128 * 128
    r = a.shape[0] // parts
    head = [dot(a, lo, mid)] if lo < mid else []
    return jnp.concatenate(
        head + [jnp.concatenate([dot(a[r * e:r * e + r], mid, hi) for e in range(parts)], axis=0)], axis=1)


def _xor_rows(x):
    hl = (lax.broadcasted_iota(jnp.int32, (32, D), 1) // DH) & 3
    m0, m1 = (hl & 1) == 0, (hl & 2) == 0
    r = [x[32 * s:32 * s + 32] for s in range(4)]
    t = [jnp.where(m0, r[s], r[s ^ 1]) for s in range(4)]
    return jnp.concatenate([jnp.where(m1, t[s], t[s ^ 2]) for s in range(4)], axis=0)


def _unpack(x):
    return pltpu.bitcast(x, BF16)


def _group_base(g):
    base = 80 * g // 64 * 64
    assert 80 * g + 80 <= base + 128 <= D and (80 * g - base) % 16 == 0
    return base


def _kernel(x_hbm, wqkv_hbm, wo_hbm, w1t_hbm, b1_hbm, w2_hbm, b2_hbm, c_hbm, wmod_hbm, o_hbm,
            x_sc, wqkv_sc, wo_sc, w1t_sc, b1_sc, w2_sc, b2_sc, c_sc, wmod_sc, sems, o_sc, osem,
            mod_sc, h_sc, q32, k32, vt32, p_sc0, p_sc1, *rest):
    ot_sc, s_sc = rest[:NFIRST], rest[NFIRST:]
    i = pl.program_id(0)
    z1 = lax.shift_right_logical(i, 20)
    z2 = lax.shift_right_logical(i, 21)

    def cols(src, dst, a, b):
        return (src.at[:, a:b], dst.at[:, a:b])

    def rows(a, b):
        return (x_hbm.at[a:b], x_sc.at[a:b])

    pairs = {
        "c": (c_hbm, c_sc),
        "x0": rows(0, 384),
        "ca": cols(wmod_hbm, wmod_sc, D, 2 * D),
        "wa": cols(wqkv_hbm, wqkv_sc, 0, C1),
        "wb": cols(wqkv_hbm, wqkv_sc, C1, C2),
        "wc": cols(wqkv_hbm, wqkv_sc, C2, 3 * D),
        "sa": cols(wmod_hbm, wmod_sc, 0, D),
        "x1": rows(384, 512),
        "modB": cols(wmod_hbm, wmod_sc, 2 * D, 5 * D),
        "wo": (wo_hbm, wo_sc),
        "b1": (b1_hbm, b1_sc),
        "b2": (b2_hbm, b2_sc),
        "w1": (w1t_hbm, w1t_sc),
        "w2": (w2_hbm, w2_sc),
        "modC": cols(wmod_hbm, wmod_sc, 5 * D, 6 * D),
        "x2": rows(512, 640),
        "x3": rows(640, S),
    }
    copies = {name: pltpu.make_async_copy(src, dst, sems.at[n])
              for n, (name, (src, dst)) in enumerate(pairs.items())}

    def wait(*names):
        for name in names:
            copies[name].wait()

    def mod(n):
        return mod_sc[0:1, n * D:(n + 1) * D]

    def compute_mod(a, b):
        c = c_sc[...].astype(F32)
        sc = jnp.broadcast_to((c * jax.nn.sigmoid(c)).astype(BF16), (16, D))
        mod_sc[:, a:b] = jnp.dot(sc, wmod_sc[:, a:b], preferred_element_type=F32)[0:8]

    def body(first):
        p_sc = p_sc0 if first else p_sc1
        p32 = p_sc.bitcast(U32)
        blk0 = 0 if first else NFIRST + (i - 1) * NSUB

        def at(bb, scale, off=0, align=8):
            v = (blk0 + bb) * scale + off
            return v if first else pl.multiple_of(v, align)

        def rows_of(bb):
            return pl.ds(at(bb, 128, align=128), 128)

        lane = lax.broadcasted_iota(jnp.int32, (16, 128), 1)
        row = lax.broadcasted_iota(jnp.int32, (16, 128), 0)
        ql = lane & 31
        tri = [row <= ql, row + 16 <= ql]
        tri32 = (jnp.where(2 * row <= ql, jnp.uint32(0xFFFF), jnp.uint32(0))
                 | jnp.where(2 * row + 1 <= ql, jnp.uint32(0xFFFF0000), jnp.uint32(0)))
        bit0 = (lane & 32) == 0
        bit1 = lane < 64
        bit0_24 = (lax.broadcasted_iota(jnp.int32, (24, 128), 1) & 32) == 0
        sub8 = lax.broadcasted_iota(jnp.int32, (8, 128), 0) < 4
        z16 = jnp.zeros((16, 128), U32)
        always = lax.broadcasted_iota(jnp.int32, (8, 128), 1) >= z1
        qcode = ((lax.broadcasted_iota(jnp.int32, (40, 128), 1) >> 5)
                 ^ (lax.broadcasted_iota(jnp.int32, (40, 128), 0) // (DH // 2)))

        def chained(fn, x, nch):
            r = x.shape[0] // nch
            outs, zero = [], None
            for e in range(nch):
                outs.append(fn(x[r * e:r * e + r], zero))
                zero = jnp.where(always, 0.0, outs[-1][0:8, 0:128])
            return jnp.concatenate(outs, axis=0)

        def ln1(rs, nch):
            return chained(lambda x, zero: _ln(x, zero) * (1.0 + mod(1)) + mod(0), x_sc[rs, :].astype(F32), nch)

        def pack(x, slot, r0=0):
            n = x.shape[0]
            p_sc[slot, r0:r0 + n, :] = x.astype(BF16)
            return p32[slot, r0 // 2:(r0 + n) // 2, :]

        def put_qkv(bb, qkv):
            qt = _xor_rows(qkv[:, 0:D] * QSCALE).T
            for t in range(5):
                q32[bb, 64 * t:64 * t + 64, :] = pack(qt[128 * t:128 * t + 128], t)
            full = jnp.concatenate([pack(qkv[:, D + 128 * t:D + 128 * t + 128], t, 128) for t in range(5)], axis=1)
            for g in range(NG):
                k32[g, pl.ds(at(bb, 64), 64), :] = full[:, _group_base(g):_group_base(g) + 128]
            vt = qkv[:, 2 * D:3 * D].T
            ones = jnp.ones((8, 128), F32)
            for hd in range(H):
                st = 8 * ((DH * hd) // 8)
                vt32[blk0 + bb, 16 * hd:16 * hd + 16, :] = pack(
                    jnp.concatenate([vt[st:st + 24], ones], axis=0), hd // 8, 32 * (hd % 8))

        hs, qkvs = {}, {}

        def qkv_stage(bb, lo, hi):
            if bb not in hs:
                hs[bb] = h_sc[...] if bb == 0 else ln1(rows_of(bb), 4).astype(BF16)
                qkvs[bb] = {}
            qkvs[bb][lo] = _dot_cols(hs[bb], wqkv_sc, lo, hi)
            if sum(v.shape[1] for v in qkvs[bb].values()) == 3 * D:
                put_qkv(bb, jnp.concatenate([qkvs[bb][k] for k in sorted(qkvs[bb])], axis=1))

        def sel(m, a, b):
            if a is None and b is None:
                return None
            return jnp.where(m, z16 if a is None else a, z16 if b is None else b)

        jobs = {}

        def stage_a(n, parts, g):
            off = 80 * g - _group_base(g)
            where, maxes = {}, {}
            used = [0] * 4
            for pi, (bb, cmin) in enumerate(parts):
                zq = q32[bb, 40 * g:40 * g + 40, :]
                for u in (range(4) if cmin == 0 else range(3, -1, -1)):
                    wts = [jnp.zeros((off // 2, 128), U32), jnp.where(qcode == u, zq, jnp.zeros_like(zq)),
                           jnp.zeros((24 - off // 2, 128), U32)]
                    qm = jnp.concatenate([w for w in wts if w.shape[0]], axis=0)
                    kmin = max(1, cmin - u)

                    def keys(r, n_):
                        return k32[g, pl.ds(at(bb, 64, 16 * u - 128 + r), n_), :]

                    mid = [keys(16 * kmin, 128 - 16 * kmin)] if kmin < 8 else []
                    if cmin == 0:
                        kk = jnp.concatenate([keys(0, 8), keys(128, 8), keys(8, 8), keys(136, 8)] + mid, axis=0)
                        s = jnp.dot(_unpack(kk), _unpack(qm), preferred_element_type=F32)
                        sm = [jnp.where(tri[0], s[16:32], s[0:16]), jnp.where(tri[1], s[48:64], s[32:48]), s[64:]]
                    else:
                        kk = jnp.concatenate([keys(128, 16)] + mid, axis=0)
                        s = jnp.dot(_unpack(kk), _unpack(qm), preferred_element_type=F32)
                        sm = [jnp.where(tri[0], s[0:16], NEG), jnp.where(tri[1], s[16:32], NEG)]
                        sm += [s[32:]] if mid else []
                    sm = jnp.concatenate(sm, axis=0)
                    nr = sm.shape[0]
                    v = u if pi == 0 else 3 - u
                    buf = s_sc[(4 * n + v) % NP]
                    buf[z1, used[v]:used[v] + nr, :] = sm
                    for j, k in enumerate([0] + list(range(kmin, 8))):
                        where[pi, u, k] = (buf, used[v] + 32 * j)
                    used[v] += nr
                    acc = [sm[0:8], sm[8:16]]
                    for r in range(2, nr // 8):
                        acc[r % 2] = jnp.maximum(acc[r % 2], sm[8 * r:8 * r + 8])
                    maxes[pi, u] = jnp.max(jnp.maximum(acc[0], acc[1]), axis=0, keepdims=True)
            jobs[n] = (parts, g, where, maxes)

        def stage_b(n, prev=None):
            parts, g, where, maxes = jobs.pop(n)
            tiles = [(pi, t) for pi, (_, cmin) in enumerate(parts) for t in (1, 0, 2) if 4 * t >= cmin]
            if len(parts) == 2:
                tiles = tiles[::-1]
            items = []
            for pi, t in tiles:
                for c in (3, 2, 1, 0):
                    for u in range(4):
                        it = (pi, u, (4 * t + c - u) % 8)
                        if 0 <= 4 * t + c - u <= 8 and it not in items:
                            items.append(it)
            assert sorted(items) == sorted(where)
            ms = {k: jnp.broadcast_to(m, (8, 128)) for k, m in maxes.items()}
            pk = {}
            step = len(parts) + 1
            for e in range(0, len(items), step):
                for pi, u, k in items[e:e + step]:
                    buf, r0 = where[pi, u, k]
                    m = ms[pi, u] if prev is None else jnp.where(always, ms[pi, u], prev)
                    p = jnp.exp2(buf[z2, r0:r0 + 32, :] - jnp.concatenate([m] * 4, axis=0))
                    pk[pi, u, k] = pack(p, 4 * pi + u, 32 * k)
                    if (pi, u, k) == items[e]:
                        nxt = p[24:32]
                prev = nxt
            ph = {}
            for pi, (bb, cmin) in enumerate(parts):
                units = []
                for u in range(4):
                    if cmin == 0:
                        last = pk[pi, u, 0] & tri32
                        head = pk[pi, u, 0] ^ last
                    else:
                        last, head = pk[pi, u, 0], None
                    chunks = [head] + [pk.get((pi, u, k)) for k in range(1, 8)] + [last]
                    units.append([None] * u + chunks + [None] * (3 - u))
                for c in range(cmin, 12):
                    u0, u1, u2, u3 = (units[u][c] for u in range(4))
                    a0, a1, a2, a3 = sel(bit0, u0, u1), sel(bit0, u1, u0), sel(bit0, u2, u3), sel(bit0, u3, u2)
                    ph[pi, 0, c] = sel(bit1, a0, a2)
                    ph[pi, 1, c] = sel(bit1, a1, a3)
                    ph[pi, 2, c] = sel(bit1, a2, a0)
                    ph[pi, 3, c] = sel(bit1, a3, a1)
            part = {}
            for pi, t in tiles:
                for hh in range(4):
                    hd = 4 * g + hh
                    pt = jnp.concatenate([ph[pi, hh, c] for c in range(4 * t, 4 * t + 4)], axis=0)
                    part[pi, hh, t] = jnp.dot(_unpack(vt32[blk0 + parts[pi][0] - 2 + t, 16 * hd:16 * hd + 16, :]),
                                              _unpack(pt), preferred_element_type=F32)
            for pi, (bb, cmin) in enumerate(parts):
                outs = []
                for hh in range(4):
                    ds = [part[pi, hh, t] for pj, t in tiles if pj == pi]
                    o = functools.reduce(jnp.add, [d[0:24] for d in ds])
                    den = functools.reduce(jnp.add, [d[24:32] for d in ds])
                    r = pl.reciprocal(den, approx=True)
                    r = r * (2.0 - den * r)
                    o = o * jnp.concatenate([r, r, r], axis=0)
                    if hh == 1:
                        o = jnp.where(bit0_24, pltpu.roll(o, 96, 1), pltpu.roll(o, 32, 1))
                    elif hh == 2:
                        o = pltpu.roll(o, 64, 1)
                    elif hh == 3:
                        o = jnp.where(bit0_24, pltpu.roll(o, 32, 1), pltpu.roll(o, 96, 1))
                    outs.append(o)
                for e in range(2):
                    oa, ob = outs[2 * e], outs[2 * e + 1]
                    pair = jnp.concatenate([oa[0:16], jnp.where(sub8, oa[16:24], ob[0:8]), ob[8:24]], axis=0)
                    ot_sc[bb][z1, 80 * g + 40 * e:80 * g + 40 * e + 40, :] = pair

        def attention(*plist, hook=None, dep=None):
            todo = [(parts, g) for parts in plist for g in range(NG)]
            stage_a(0, *todo[0])
            for n in range(len(todo) - 1):
                stage_a(n + 1, *todo[n + 1])
                if hook is not None and n == len(todo) - 2:
                    hook()
                stage_b(n, dep if n == 0 else None)
            return functools.partial(stage_b, len(todo) - 1)

        x1s, ys, gs = {}, {}, {}

        def wo_stage(bb, halves=False, nch=1):
            o = ot_sc[bb][z2].T
            if halves:
                attn = jnp.concatenate([_dot_cols(o[64 * e:64 * e + 64], wo_sc, 0, D, 2) for e in range(2)], axis=0)
            else:
                attn = _dot_cols(o, wo_sc, 0, D, 4)
            x1s[bb] = x_sc[rows_of(bb), :].astype(F32) + mod(2) * attn
            ys[bb] = chained(lambda x, zero: _ln(_ln(x, zero) * (1.0 + mod(4)) + mod(3)), x1s[bb], nch)

        def w1_stage(bb, between=None, after=None):
            y = ys[bb]
            if between is None:
                head = _dot_cols(y, w1t_sc, 0, 768, nt=True)
            else:
                head = _dot_cols(y, w1t_sc, 0, 512, nt=True)
                between()
                head = jnp.concatenate([head, _dot_cols(y, w1t_sc, 512, 768, nt=True)], axis=1)
            fm = F - 64
            tail = (lax.dot_general(w1t_sc[fm:F, 0:512], y[:, 0:512].astype(BF16), NT, preferred_element_type=F32).T
                    + lax.dot_general(y[:, 512:D].astype(BF16), w1t_sc[fm:F, 512:D], NT, preferred_element_type=F32))
            h1 = jnp.concatenate([head, _dot_cols(y, w1t_sc, 768, fm, nt=True), tail], axis=1)
            h1 = h1 + b1_sc[...].astype(F32).reshape(1, F)
            if after is None:
                gs[bb] = _gelu(h1)
            else:
                g = [_gelu(h1[:, 0:fm - 256]), None, _gelu(h1[:, fm:F])]
                after()
                g[1] = _gelu(h1[:, fm - 256:fm])
                gs[bb] = jnp.concatenate(g, axis=1)

        def w2_stage(bb, lo=0, hi=D, parts=1, with_mod=False):
            b2 = b2_sc[...].astype(F32).reshape(1, D)
            mlp = _dot_cols(gs[bb], w2_sc, lo, hi, parts) + b2[:, lo:hi]
            if with_mod:
                compute_mod(5 * D + lo, 5 * D + hi)
            gb = mod_sc[0:1, 5 * D + lo:5 * D + hi]
            o_sc[rows_of(bb), lo:hi] = (x1s[bb][:, lo:hi] + gb * mlp).astype(o_sc.dtype)

        def flush(bb, lo=0, hi=D):
            pltpu.make_async_copy(o_sc.at[rows_of(bb), lo:hi], o_hbm.at[rows_of(bb), lo:hi], osem).start()

        if first:
            for cp in copies.values():
                cp.start()
            wait("c", "x0")
            xn = _ln(x_sc[0:384, :].astype(F32))
            wait("ca")
            compute_mod(D, 2 * D)
            t = [xn[128 * bb:128 * bb + 128] * (1.0 + mod(1)) for bb in range(3)]
            res = [[], [], []]
            wait("wa")
            for bb in range(3):
                res[bb].append(_dot_cols(t[bb], wqkv_sc, 0, C1, 4 if bb == 2 else 1))
            wait("wb")
            for bb in range(3):
                res[bb].append(_dot_cols(t[bb], wqkv_sc, C1, C2, 4 if bb == 2 else 1))
            wait("wc")
            for bb in range(2):
                res[bb].append(_dot_cols(t[bb], wqkv_sc, C2, 3 * D, 2 if bb == 1 else 1))
            wait("sa", "x1")
            for c0 in range(0, D, 128):
                res[2].append(_dot_cols(t[2], wqkv_sc, C2 + c0, C2 + c0 + 128))
                compute_mod(c0, c0 + 128)
            res[2].append(_dot_cols(t[2], wqkv_sc, C2 + D, 3 * D))
            h3 = ln1(rows_of(3), 1)
            sa = jnp.broadcast_to(mod(0), (16, D))
            r3 = jnp.concatenate(
                [_dot_cols(jnp.concatenate([h3, sa], axis=0), wqkv_sc, 0, QE),
                 jnp.concatenate([_dot_cols(h3, wqkv_sc, QE, 3 * D, 4), _dot_cols(sa, wqkv_sc, QE, 3 * D)], axis=0)],
                axis=1)
            for bb in range(4):
                put_qkv(bb, r3[0:128] if bb == 3 else jnp.concatenate(res[bb], axis=1) + r3[128:129])

            def mid_weights():
                wait("modB", "wo", "b1", "b2", "w1")
                compute_mod(2 * D, 4 * D)

            fin = attention([(1, 4), (0, 8)], [(2, 0)], hook=mid_weights)
            compute_mod(4 * D, 5 * D)
            fin()
            wo_stage(0)
            wo_stage(1)
            wo_stage(2)
            w1_stage(0)
            fin = attention([(3, 0)])
            w1_stage(1, fin, functools.partial(wait, "w2", "modC", "x2"))
            for c0 in range(0, D, 128):
                w2_stage(0, c0, c0 + 128, with_mod=True)
                if c0 == 0:
                    wo_stage(3, halves=True)
            flush(0)
            w1_stage(2)
            w2_stage(1)
            flush(1)
            w1_stage(3)
            w2_stage(2)
            flush(2)
            h_sc[...] = ln1(rows_of(NFIRST), 8).astype(BF16)
            w2_stage(3, parts=2)
            flush(3)
        else:
            qkv_stage(0, 0, 3 * D)
            qkv_stage(1, QE, 3 * D)
            fin = attention([(0, 0)])
            qkv_stage(1, 0, 512)
            fin()
            qkv_stage(1, 512, 2 * D)
            wo_stage(0)
            qkv_stage(1, 2 * D, QE)
            y0 = functools.reduce(jnp.maximum, [ys[0][8 * r:8 * r + 8, 0:128] for r in range(16)])
            fin = attention([(1, 0)], dep=y0)
            w1_stage(0, fin)
            wo_stage(1, nch=4)
            w2_stage(0)
            w1_stage(1)
            flush(0)
            nxt = pl.multiple_of(jnp.minimum(blk0 + NSUB, S // 128 - 1) * 128, 128)
            h_sc[...] = ln1(pl.ds(nxt, 128), 8).astype(BF16)
            w2_stage(1, 0, 512)
            flush(1, 0, 512)
            w2_stage(1, 512, D, 2)
            flush(1, 512, D)

    pl.when(i == 1)(functools.partial(wait, "x3"))
    pl.when(i == 0)(functools.partial(body, True))
    pl.when(i > 0)(functools.partial(body, False))

    @pl.when(i == NSTEP - 1)
    def _():
        pltpu.make_async_copy(o_sc, o_hbm, osem).wait()


@jax.jit
def pallas_adaLN_cond__sliding_block__mixer_channel_mlp__prompt_kernel(
    A_x, A_wqkv, A_wo, B_x, B_w1, B_b1, B_w2, B_b2, c, w_mod):
    del B_x
    out = pl.pallas_call(
        _kernel,
        grid=(NSTEP,),
        in_specs=[pl.BlockSpec(memory_space=pl.ANY)] * 9,
        out_specs=pl.BlockSpec(memory_space=pl.ANY),
        out_shape=jax.ShapeDtypeStruct((S, D), A_x.dtype),
        scratch_shapes=[
            pltpu.VMEM((S, D), BF16),
            pltpu.VMEM((D, 3 * D), BF16),
            pltpu.VMEM((D, D), BF16),
            pltpu.VMEM((F, D), BF16),
            pltpu.VMEM((F,), BF16),
            pltpu.VMEM((F, D), BF16),
            pltpu.VMEM((D,), BF16),
            pltpu.VMEM((1, D), BF16),
            pltpu.VMEM((D, 6 * D), BF16),
            pltpu.SemaphoreType.DMA((17,)),
            pltpu.VMEM((S, D), BF16),
            pltpu.SemaphoreType.DMA(()),
            pltpu.VMEM((8, 6 * D), F32),
            pltpu.VMEM((128, D), BF16),
            pltpu.VMEM((NFIRST, D // 2, 128), U32),
            pltpu.VMEM((NG, S // 2, 128), U32),
            pltpu.VMEM((S // 128, H * 16, 128), U32),
            pltpu.VMEM((8, 256, 128), BF16),
            pltpu.VMEM((8, 256, 128), BF16),
        ] + [pltpu.VMEM((1, D, 128), F32)] * NFIRST
          + [pltpu.VMEM((1, 288, 128), F32)] * NP,
        compiler_params=pltpu.CompilerParams(
            dimension_semantics=("arbitrary",), vmem_limit_bytes=100 * 1024 * 1024,
            disable_bounds_checks=True, disable_semaphore_checks=True),
        name="fused_block",
    )(A_x.reshape(S, D), A_wqkv, A_wo, B_w1.T, B_b1, B_w2, B_b2, c, w_mod)
    return out.reshape(1, S, D)
```

```python
import functools

import jax
import jax.numpy as jnp
from jax import lax
import jax.experimental.pallas as pl
import jax.experimental.pallas.tpu as pltpu

S = 2048
D = 640
H = 32
DH = 20
F = 1728
NFIRST = 4
NSUB = 2
NSTEP = 1 + (S // 128 - NFIRST) // NSUB
NG = H // 4
NP = 8
C1, C2 = 384, 1024
QE = 3 * D - 128
EPS = 1e-5
NEG = -1e30
F32 = jnp.float32
BF16 = jnp.bfloat16
U32 = jnp.uint32
QSCALE = (DH ** -0.5) * 1.4426950408889634
NT = (((1,), (1,)), ((), ()))


def _rowsum(x, zero=None):
    t = x[:, 0:128]
    for j in range(1, D // 128):
        t = t + x[:, 128 * j:128 * j + 128]
    if zero is not None:
        t = t + jnp.concatenate([zero] * (x.shape[0] // 8), axis=0)
    return jnp.sum(t, axis=-1, keepdims=True)


def _ln(x, zero=None):
    xc = x - _rowsum(x, zero) * (1.0 / D)
    v = _rowsum(xc * xc) * (1.0 / D)
    return xc * lax.rsqrt(v + EPS)


def _gelu(x):
    c1 = 0.7978845608028654
    c2 = c1 * 0.044715
    u = x * (c1 + c2 * (x * x))
    return (0.5 * x) * (1.0 + jnp.tanh(u))


def _dot_cols(a, w_ref, lo, hi, parts=1, nt=False):
    def dot(x, c0, c1):
        x = x.astype(BF16)
        if nt:
            return lax.dot_general(x, w_ref[c0:c1, :], NT, preferred_element_type=F32)
        return jnp.dot(x, w_ref[:, c0:c1], preferred_element_type=F32)
    if parts == 1:
        return dot(a, lo, hi)
    mid = (hi - 1) // 128 * 128
    r = a.shape[0] // parts
    head = [dot(a, lo, mid)] if lo < mid else []
    return jnp.concatenate(
        head + [jnp.concatenate([dot(a[r * e:r * e + r], mid, hi) for e in range(parts)], axis=0)], axis=1)


def _xor_rows(x):
    hl = (lax.broadcasted_iota(jnp.int32, (32, D), 1) // DH) & 3
    m0, m1 = (hl & 1) == 0, (hl & 2) == 0
    r = [x[32 * s:32 * s + 32] for s in range(4)]
    t = [jnp.where(m0, r[s], r[s ^ 1]) for s in range(4)]
    return jnp.concatenate([jnp.where(m1, t[s], t[s ^ 2]) for s in range(4)], axis=0)


def _unpack(x):
    return pltpu.bitcast(x, BF16)


def _group_base(g):
    base = 80 * g // 64 * 64
    assert 80 * g + 80 <= base + 128 <= D and (80 * g - base) % 16 == 0
    return base


def _kernel(x_hbm, wqkv_hbm, wo_hbm, w1t_hbm, b1_hbm, w2_hbm, b2_hbm, c_hbm, wmod_hbm, o_hbm,
            sems, osem, x_sc, wqkv_sc, wo_sc, w1t_sc, w2_sc, wmod_sc, o_sc,
            h_sc, q32, k32, vt32, p_sc0, p_sc1, mod_sc, *rest):
    ot_sc, s_sc = rest[:NFIRST], rest[NFIRST:NFIRST + NP]
    silu_sc, b1_sc, b2_sc, c_sc = rest[NFIRST + NP:]
    i = pl.program_id(0)
    z1 = lax.shift_right_logical(i, 20)
    z2 = lax.shift_right_logical(i, 21)

    def cols(src, dst, a, b):
        return (src.at[:, a:b], dst.at[:, a:b])

    def rows(a, b):
        return (x_hbm.at[a:b], x_sc.at[a:b])

    pairs = {
        "c": (c_hbm, c_sc),
        "x0": rows(0, 384),
        "ca": cols(wmod_hbm, wmod_sc, D, 2 * D),
        "wa": cols(wqkv_hbm, wqkv_sc, 0, C1),
        "wb": cols(wqkv_hbm, wqkv_sc, C1, C2),
        "wc": cols(wqkv_hbm, wqkv_sc, C2, 3 * D),
        "sa": cols(wmod_hbm, wmod_sc, 0, D),
        "x1": rows(384, 512),
        "modB": cols(wmod_hbm, wmod_sc, 2 * D, 5 * D),
        "wo": (wo_hbm, wo_sc),
        "b1": (b1_hbm, b1_sc),
        "b2": (b2_hbm, b2_sc),
        "w1": (w1t_hbm, w1t_sc),
        "w2": (w2_hbm, w2_sc),
        "modC": cols(wmod_hbm, wmod_sc, 5 * D, 6 * D),
        "x2": rows(512, 640),
        "x3": rows(640, S),
    }
    copies = {name: pltpu.make_async_copy(src, dst, sems.at[n])
              for n, (name, (src, dst)) in enumerate(pairs.items())}

    def wait(*names):
        for name in names:
            copies[name].wait()

    def mod(n):
        return mod_sc[0:1, n * D:(n + 1) * D]

    def compute_mod(a, b):
        mod_sc[:, a:b] = jnp.dot(silu_sc[...], wmod_sc[:, a:b], preferred_element_type=F32)[0:8]

    def body(first):
        p_sc = p_sc0 if first else p_sc1
        p32 = p_sc.bitcast(U32)
        blk0 = 0 if first else NFIRST + (i - 1) * NSUB

        base = {scale: 0 if first else pl.multiple_of(blk0 * scale, scale) for scale in (64, 128)}

        def at(bb, scale, off=0):
            return base[scale] + (bb * scale + off)

        def rows_of(bb):
            return pl.ds(at(bb, 128), 128)

        lane = lax.broadcasted_iota(jnp.int32, (16, 128), 1)
        row = lax.broadcasted_iota(jnp.int32, (16, 128), 0)
        ql = lane & 31
        tri = [row <= ql, row + 16 <= ql]
        tri32 = (jnp.where(2 * row <= ql, jnp.uint32(0xFFFF), jnp.uint32(0))
                 | jnp.where(2 * row + 1 <= ql, jnp.uint32(0xFFFF0000), jnp.uint32(0)))
        bit0 = (lane & 32) == 0
        bit1 = lane < 64
        bit0_24 = (lax.broadcasted_iota(jnp.int32, (24, 128), 1) & 32) == 0
        sub8 = lax.broadcasted_iota(jnp.int32, (8, 128), 0) < 4
        z16 = jnp.zeros((16, 128), U32)
        always = lax.broadcasted_iota(jnp.int32, (8, 128), 1) >= z1
        qcode = ((lax.broadcasted_iota(jnp.int32, (40, 128), 1) >> 5)
                 ^ (lax.broadcasted_iota(jnp.int32, (40, 128), 0) // (DH // 2)))

        def chained(fn, x, nch):
            r = x.shape[0] // nch
            outs, zero = [], None
            for e in range(nch):
                if outs:
                    zero = jnp.where(always, 0.0, outs[-1][0:8, 0:128])
                outs.append(fn(x[r * e:r * e + r], zero))
            return jnp.concatenate(outs, axis=0)

        def ln1(rs, nch):
            return chained(lambda x, zero: _ln(x, zero) * (1.0 + mod(1)) + mod(0), x_sc[rs, :].astype(F32), nch)

        def pack(x, slot, r0=0):
            n = x.shape[0]
            p_sc[slot, r0:r0 + n, :] = x.astype(BF16)
            return p32[slot, r0 // 2:(r0 + n) // 2, :]

        def put_qkv(bb, qkv):
            qt = _xor_rows(qkv[:, 0:D] * QSCALE).T
            for t in range(5):
                q32[bb, 64 * t:64 * t + 64, :] = pack(qt[128 * t:128 * t + 128], t)
            full = jnp.concatenate([pack(qkv[:, D + 128 * t:D + 128 * t + 128], t, 128) for t in range(5)], axis=1)
            for g in range(NG):
                k32[g, pl.ds(at(bb, 64), 64), :] = full[:, _group_base(g):_group_base(g) + 128]
            vt = qkv[:, 2 * D:3 * D].T
            ones = jnp.ones((8, 128), F32)
            for hd in range(H):
                st = 8 * ((DH * hd) // 8)
                vt32[blk0 + bb, 16 * hd:16 * hd + 16, :] = pack(
                    jnp.concatenate([vt[st:st + 24], ones], axis=0), hd // 8, 32 * (hd % 8))

        hs, qkvs = {}, {}

        def qkv_stage(bb, lo, hi):
            if bb not in hs:
                hs[bb] = h_sc[...] if bb == 0 else ln1(rows_of(bb), 4).astype(BF16)
                qkvs[bb] = {}
            qkvs[bb][lo] = _dot_cols(hs[bb], wqkv_sc, lo, hi)
            if sum(v.shape[1] for v in qkvs[bb].values()) == 3 * D:
                put_qkv(bb, jnp.concatenate([qkvs[bb][k] for k in sorted(qkvs[bb])], axis=1))

        def sel(m, a, b):
            if a is None and b is None:
                return None
            return jnp.where(m, z16 if a is None else a, z16 if b is None else b)

        jobs = {}

        def stage_a(n, parts, g):
            off = 80 * g - _group_base(g)
            where, maxes = {}, {}
            used = [0] * 4
            for pi, (bb, cmin) in enumerate(parts):
                zq = q32[bb, 40 * g:40 * g + 40, :]
                for u in (range(4) if cmin == 0 else range(3, -1, -1)):
                    z8 = jnp.zeros((8, 128), U32)
                    qm = jnp.concatenate([z8] * (off // 16) + [jnp.where(qcode == u, zq, jnp.zeros_like(zq))]
                                         + [z8] * (3 - off // 16), axis=0)
                    kmin = max(1, cmin - u)

                    def keys(r, n_):
                        return k32[g, pl.ds(at(bb, 64, 16 * u - 128 + r), n_), :]

                    mid = [keys(16 * kmin, 128 - 16 * kmin)] if kmin < 8 else []
                    if cmin == 0:
                        kk = jnp.concatenate([keys(0, 8), keys(128, 8), keys(8, 8), keys(136, 8)] + mid, axis=0)
                        s = jnp.dot(_unpack(kk), _unpack(qm), preferred_element_type=F32)
                        sm = [jnp.where(tri[0], s[16:32], s[0:16]), jnp.where(tri[1], s[48:64], s[32:48]), s[64:]]
                    else:
                        kk = jnp.concatenate([keys(128, 16)] + mid, axis=0)
                        s = jnp.dot(_unpack(kk), _unpack(qm), preferred_element_type=F32)
                        sm = [jnp.where(tri[0], s[0:16], NEG), jnp.where(tri[1], s[16:32], NEG)]
                        sm += [s[32:]] if mid else []
                    sm = jnp.concatenate(sm, axis=0)
                    nr = sm.shape[0]
                    v = u if pi == 0 else 3 - u
                    buf = s_sc[(4 * n + v) % NP]
                    buf[z1, used[v]:used[v] + nr, :] = sm
                    for j, k in enumerate([0] + list(range(kmin, 8))):
                        where[pi, u, k] = (buf, used[v] + 32 * j)
                    used[v] += nr
                    acc = [sm[0:8], sm[8:16]]
                    for r in range(2, nr // 8):
                        acc[r % 2] = jnp.maximum(acc[r % 2], sm[8 * r:8 * r + 8])
                    maxes[pi, u] = jnp.max(jnp.maximum(acc[0], acc[1]), axis=0, keepdims=True)
            jobs[n] = (parts, g, where, maxes)

        def stage_b(n, prev=None):
            parts, g, where, maxes = jobs.pop(n)
            tiles = [(pi, t) for pi, (_, cmin) in enumerate(parts) for t in (1, 0, 2) if 4 * t >= cmin]
            if len(parts) == 2:
                tiles = tiles[::-1]
            items = []
            for pi, t in tiles:
                for c in (3, 2, 1, 0):
                    for u in range(4):
                        it = (pi, u, (4 * t + c - u) % 8)
                        if 0 <= 4 * t + c - u <= 8 and it not in items:
                            items.append(it)
            assert sorted(items) == sorted(where)
            ms = {k: jnp.broadcast_to(m, (8, 128)) for k, m in maxes.items()}
            pk = {}
            step = len(parts) + 1
            for e in range(0, len(items), step):
                for pi, u, k in items[e:e + step]:
                    buf, r0 = where[pi, u, k]
                    m = ms[pi, u] if prev is None else jnp.where(always, ms[pi, u], prev)
                    p = jnp.exp2(buf[z2, r0:r0 + 32, :] - jnp.concatenate([m] * 4, axis=0))
                    pk[pi, u, k] = pack(p, 4 * pi + u, 32 * k)
                    if (pi, u, k) == items[e]:
                        nxt = p[24:32]
                prev = nxt
            ph = {}
            for pi, (bb, cmin) in enumerate(parts):
                units = []
                for u in range(4):
                    if cmin == 0:
                        last = pk[pi, u, 0] & tri32
                        head = pk[pi, u, 0] ^ last
                    else:
                        last, head = pk[pi, u, 0], None
                    chunks = [head] + [pk.get((pi, u, k)) for k in range(1, 8)] + [last]
                    units.append([None] * u + chunks + [None] * (3 - u))
                for c in range(cmin, 12):
                    u0, u1, u2, u3 = (units[u][c] for u in range(4))
                    a0, a1, a2, a3 = sel(bit0, u0, u1), sel(bit0, u1, u0), sel(bit0, u2, u3), sel(bit0, u3, u2)
                    ph[pi, 0, c] = sel(bit1, a0, a2)
                    ph[pi, 1, c] = sel(bit1, a1, a3)
                    ph[pi, 2, c] = sel(bit1, a2, a0)
                    ph[pi, 3, c] = sel(bit1, a3, a1)
            part = {}
            for pi, t in tiles:
                for hh in range(4):
                    hd = 4 * g + hh
                    pt = jnp.concatenate([ph[pi, hh, c] for c in range(4 * t, 4 * t + 4)], axis=0)
                    part[pi, hh, t] = jnp.dot(_unpack(vt32[blk0 + parts[pi][0] - 2 + t, 16 * hd:16 * hd + 16, :]),
                                              _unpack(pt), preferred_element_type=F32)
            for pi, (bb, cmin) in enumerate(parts):
                outs = []
                for hh in range(4):
                    ds = [part[pi, hh, t] for pj, t in tiles if pj == pi]
                    o = functools.reduce(jnp.add, [d[0:24] for d in ds])
                    den = functools.reduce(jnp.add, [d[24:32] for d in ds])
                    r = pl.reciprocal(den, approx=True)
                    r = r * (2.0 - den * r)
                    o = o * jnp.concatenate([r, r, r], axis=0)
                    if hh == 1:
                        o = jnp.where(bit0_24, pltpu.roll(o, 96, 1), pltpu.roll(o, 32, 1))
                    elif hh == 2:
                        o = pltpu.roll(o, 64, 1)
                    elif hh == 3:
                        o = jnp.where(bit0_24, pltpu.roll(o, 32, 1), pltpu.roll(o, 96, 1))
                    outs.append(o)
                for e in range(2):
                    oa, ob = outs[2 * e], outs[2 * e + 1]
                    pair = jnp.concatenate([oa[0:16], jnp.where(sub8, oa[16:24], ob[0:8]), ob[8:24]], axis=0)
                    ot_sc[bb][z1, 80 * g + 40 * e:80 * g + 40 * e + 40, :] = pair

        def attention(*plist, hook=None, dep=None):
            todo = [(parts, g) for parts in plist for g in range(NG)]
            stage_a(0, *todo[0])
            for n in range(len(todo) - 1):
                stage_a(n + 1, *todo[n + 1])
                if hook is not None and n == len(todo) - 2:
                    hook()
                stage_b(n, dep if n == 0 else None)
            return functools.partial(stage_b, len(todo) - 1)

        x1s, ys, gs = {}, {}, {}

        def wo_stage(bb, halves=False, nch=1):
            o = ot_sc[bb][z2].T
            if halves:
                attn = jnp.concatenate([_dot_cols(o[64 * e:64 * e + 64], wo_sc, 0, D, 2) for e in range(2)], axis=0)
            else:
                attn = _dot_cols(o, wo_sc, 0, D, 4)
            x1s[bb] = x_sc[rows_of(bb), :].astype(F32) + mod(2) * attn
            ys[bb] = chained(lambda x, zero: _ln(_ln(x, zero) * (1.0 + mod(4)) + mod(3)), x1s[bb], nch)

        def w1_stage(bb, between=None, after=None):
            y = ys[bb]
            if between is None:
                head = _dot_cols(y, w1t_sc, 0, 768, nt=True)
            else:
                head = _dot_cols(y, w1t_sc, 0, 512, nt=True)
                between()
                head = jnp.concatenate([head, _dot_cols(y, w1t_sc, 512, 768, nt=True)], axis=1)
            fm = F - 64
            tail = (lax.dot_general(w1t_sc[fm:F, 0:512], y[:, 0:512].astype(BF16), NT, preferred_element_type=F32).T
                    + lax.dot_general(y[:, 512:D].astype(BF16), w1t_sc[fm:F, 512:D], NT, preferred_element_type=F32))
            h1 = jnp.concatenate([head, _dot_cols(y, w1t_sc, 768, fm, nt=True), tail], axis=1)
            h1 = h1 + b1_sc[...].astype(F32).reshape(1, F)
            if after is None:
                gs[bb] = _gelu(h1)
            else:
                g = [_gelu(h1[:, 0:fm - 256]), None, _gelu(h1[:, fm:F])]
                after()
                g[1] = _gelu(h1[:, fm - 256:fm])
                gs[bb] = jnp.concatenate(g, axis=1)

        def w2_stage(bb, lo=0, hi=D, parts=1, with_mod=False):
            b2 = b2_sc[...].astype(F32).reshape(1, D)
            mlp = _dot_cols(gs[bb], w2_sc, lo, hi, parts) + b2[:, lo:hi]
            if with_mod:
                compute_mod(5 * D + lo, 5 * D + hi)
            gb = mod_sc[0:1, 5 * D + lo:5 * D + hi]
            o_sc[rows_of(bb), lo:hi] = (x1s[bb][:, lo:hi] + gb * mlp).astype(o_sc.dtype)

        def flush(bb, lo=0, hi=D):
            pltpu.make_async_copy(o_sc.at[rows_of(bb), lo:hi], o_hbm.at[rows_of(bb), lo:hi], osem).start()

        if first:
            for cp in copies.values():
                cp.start()
            wait("c", "x0")
            c = c_sc[...].astype(F32)
            silu_sc[...] = jnp.broadcast_to(c * jax.nn.sigmoid(c), (16, D)).astype(BF16)
            xn = _ln(x_sc[0:384, :].astype(F32))
            wait("ca")
            compute_mod(D, 2 * D)
            t = [xn[128 * bb:128 * bb + 128] * (1.0 + mod(1)) for bb in range(3)]
            res = [[], [], []]
            wait("wa")
            for bb in range(3):
                res[bb].append(_dot_cols(t[bb], wqkv_sc, 0, C1, 4 if bb == 2 else 1))
            wait("wb")
            for bb in range(3):
                res[bb].append(_dot_cols(t[bb], wqkv_sc, C1, C2, 4 if bb == 2 else 1))
            wait("wc")
            for bb in range(2):
                res[bb].append(_dot_cols(t[bb], wqkv_sc, C2, 3 * D, 2 if bb == 1 else 1))
            wait("sa", "x1")
            for c0 in range(0, D, 128):
                res[2].append(_dot_cols(t[2], wqkv_sc, C2 + c0, C2 + c0 + 128))
                compute_mod(c0, c0 + 128)
            res[2].append(_dot_cols(t[2], wqkv_sc, C2 + D, 3 * D))
            h3 = ln1(rows_of(3), 1)
            sa = jnp.broadcast_to(mod(0), (16, D))
            r3 = jnp.concatenate(
                [_dot_cols(jnp.concatenate([h3, sa], axis=0), wqkv_sc, 0, QE),
                 jnp.concatenate([_dot_cols(h3, wqkv_sc, QE, 3 * D, 4), _dot_cols(sa, wqkv_sc, QE, 3 * D)], axis=0)],
                axis=1)
            for bb in range(4):
                put_qkv(bb, r3[0:128] if bb == 3 else jnp.concatenate(res[bb], axis=1) + r3[128:129])

            def mid_weights():
                wait("modB", "wo", "b1", "b2", "w1")
                compute_mod(2 * D, 4 * D)

            fin = attention([(1, 4), (0, 8)], [(2, 0)], hook=mid_weights)
            compute_mod(4 * D, 5 * D)
            fin()
            wo_stage(0)
            wo_stage(1)
            wo_stage(2)
            w1_stage(0)
            fin = attention([(3, 0)])
            w1_stage(1, fin, functools.partial(wait, "w2", "modC", "x2"))
            for c0 in range(0, D, 128):
                w2_stage(0, c0, c0 + 128, with_mod=True)
                if c0 == 0:
                    wo_stage(3, halves=True)
            flush(0)
            w1_stage(2)
            w2_stage(1)
            flush(1)
            w1_stage(3)
            w2_stage(2)
            flush(2)
            h_sc[...] = ln1(rows_of(NFIRST), 8).astype(BF16)
            w2_stage(3, parts=2)
            flush(3)
        else:
            qkv_stage(0, 0, 3 * D)
            qkv_stage(1, QE, 3 * D)
            fin = attention([(0, 0)])
            qkv_stage(1, 0, 512)
            fin()
            qkv_stage(1, 512, 2 * D)
            wo_stage(0)
            qkv_stage(1, 2 * D, QE)
            y0 = functools.reduce(jnp.maximum, [ys[0][8 * r:8 * r + 8, 0:128] for r in range(16)])
            fin = attention([(1, 0)], dep=y0)
            w1_stage(0, fin)
            wo_stage(1, nch=4)
            w2_stage(0)
            w1_stage(1)
            flush(0)
            nxt = pl.multiple_of(jnp.minimum(blk0 + NSUB, S // 128 - 1) * 128, 128)
            h_sc[...] = ln1(pl.ds(nxt, 128), 8).astype(BF16)
            w2_stage(1, 0, 512)
            flush(1, 0, 512)
            w2_stage(1, 512, D, 2)
            flush(1, 512, D)

    pl.when(i == 1)(functools.partial(wait, "x3"))
    pl.when(i == 0)(functools.partial(body, True))
    pl.when(i > 0)(functools.partial(body, False))

    @pl.when(i == NSTEP - 1)
    def _():
        pltpu.make_async_copy(o_sc, o_hbm, osem).wait()


@jax.jit
def pallas_adaLN_cond__sliding_block__mixer_channel_mlp__prompt_kernel(
    A_x, A_wqkv, A_wo, B_x, B_w1, B_b1, B_w2, B_b2, c, w_mod):
    del B_x
    out = pl.pallas_call(
        _kernel,
        grid=(NSTEP,),
        in_specs=[pl.BlockSpec(memory_space=pl.ANY)] * 9,
        out_specs=pl.BlockSpec(memory_space=pl.ANY),
        out_shape=jax.ShapeDtypeStruct((S, D), A_x.dtype),
        scratch_shapes=[
            pltpu.SemaphoreType.DMA((17,)),
            pltpu.SemaphoreType.DMA(()),
            pltpu.VMEM((S, D), BF16),
            pltpu.VMEM((D, 3 * D), BF16),
            pltpu.VMEM((D, D), BF16),
            pltpu.VMEM((F, D), BF16),
            pltpu.VMEM((F, D), BF16),
            pltpu.VMEM((D, 6 * D), BF16),
            pltpu.VMEM((S, D), BF16),
            pltpu.VMEM((128, D), BF16),
            pltpu.VMEM((NFIRST, D // 2, 128), U32),
            pltpu.VMEM((NG, S // 2, 128), U32),
            pltpu.VMEM((S // 128, H * 16, 128), U32),
            pltpu.VMEM((8, 256, 128), BF16),
            pltpu.VMEM((8, 256, 128), BF16),
            pltpu.VMEM((8, 4096), F32),
        ] + [pltpu.VMEM((1, D, 128), F32)] * NFIRST
          + [pltpu.VMEM((1, 288, 128), F32)] * NP
          + [pltpu.VMEM((16, D), BF16),
             pltpu.VMEM((F,), BF16),
             pltpu.VMEM((D,), BF16),
             pltpu.VMEM((1, D), BF16)],
        compiler_params=pltpu.CompilerParams(
            dimension_semantics=("arbitrary",), vmem_limit_bytes=100 * 1024 * 1024,
            disable_bounds_checks=True, disable_semaphore_checks=True),
        name="fused_block",
    )(A_x.reshape(S, D), A_wqkv, A_wo, B_w1.T, B_b1, B_w2, B_b2, c, w_mod)
    return out.reshape(1, S, D)
```

```python
import functools

import jax
import jax.numpy as jnp
from jax import lax
import jax.experimental.pallas as pl
import jax.experimental.pallas.tpu as pltpu

S = 2048
D = 640
H = 32
DH = 20
F = 1728
NFIRST = 4
NSUB = 2
NSTEP = 1 + (S // 128 - NFIRST) // NSUB
NG = H // 4
NP = 8
C1, C2 = 384, 1024
QE = 3 * D - 128
EPS = 1e-5
NEG = -1e30
F32 = jnp.float32
BF16 = jnp.bfloat16
U32 = jnp.uint32
QSCALE = (DH ** -0.5) * 1.4426950408889634
NT = (((1,), (1,)), ((), ()))


def _rowsum(x, zero=None):
    t = x[:, 0:128]
    for j in range(1, D // 128):
        t = t + x[:, 128 * j:128 * j + 128]
    if zero is not None:
        t = t + jnp.concatenate([zero] * (x.shape[0] // 8), axis=0)
    return jnp.sum(t, axis=-1, keepdims=True)


def _ln(x, zero=None):
    xc = x - _rowsum(x, zero) * (1.0 / D)
    v = _rowsum(xc * xc) * (1.0 / D)
    return xc * lax.rsqrt(v + EPS)


def _gelu(x):
    c1 = 0.7978845608028654
    c2 = c1 * 0.044715
    u = x * (c1 + c2 * (x * x))
    return (0.5 * x) * (1.0 + jnp.tanh(u))


def _dot_cols(a, w_ref, lo, hi, parts=1, nt=False):
    def dot(x, c0, c1):
        x = x.astype(BF16)
        if nt:
            return lax.dot_general(x, w_ref[c0:c1, :], NT, preferred_element_type=F32)
        return jnp.dot(x, w_ref[:, c0:c1], preferred_element_type=F32)
    if parts == 1:
        return dot(a, lo, hi)
    mid = (hi - 1) // 128 * 128
    r = a.shape[0] // parts
    head = [dot(a, lo, mid)] if lo < mid else []
    return jnp.concatenate(
        head + [jnp.concatenate([dot(a[r * e:r * e + r], mid, hi) for e in range(parts)], axis=0)], axis=1)


def _xor_rows(x):
    hl = (lax.broadcasted_iota(jnp.int32, (32, D), 1) // DH) & 3
    m0, m1 = (hl & 1) == 0, (hl & 2) == 0
    r = [x[32 * s:32 * s + 32] for s in range(4)]
    t = [jnp.where(m0, r[s], r[s ^ 1]) for s in range(4)]
    return jnp.concatenate([jnp.where(m1, t[s], t[s ^ 2]) for s in range(4)], axis=0)


def _unpack(x):
    return pltpu.bitcast(x, BF16)


def _group_base(g):
    base = 80 * g // 64 * 64
    assert 80 * g + 80 <= base + 128 <= D and (80 * g - base) % 16 == 0
    return base


def _kernel(x_hbm, wqkv_hbm, wo_hbm, w1t_hbm, b1_hbm, w2_hbm, b2_hbm, c_hbm, wmod_hbm, o_hbm,
            sems, osem, x_sc, wqkv_sc, wo_sc, w1t_sc, w2_sc, wmod_sc, o_sc,
            h_sc, q32, k32, vt32, p_sc0, p_sc1, mod_sc, *rest):
    ot_sc, s_sc = rest[:NFIRST], rest[NFIRST:NFIRST + NP]
    silu_sc, b1_sc, b2_sc, c_sc = rest[NFIRST + NP:]
    i = pl.program_id(0)
    z1 = lax.shift_right_logical(i, 20)
    z2 = lax.shift_right_logical(i, 21)

    def cols(src, dst, a, b):
        return (src.at[:, a:b], dst.at[:, a:b])

    def rows(a, b):
        return (x_hbm.at[a:b], x_sc.at[a:b])

    pairs = {
        "c": (c_hbm, c_sc),
        "x0": rows(0, 384),
        "ca": cols(wmod_hbm, wmod_sc, D, 2 * D),
        "wa": cols(wqkv_hbm, wqkv_sc, 0, C1),
        "wb": cols(wqkv_hbm, wqkv_sc, C1, C2),
        "wc": cols(wqkv_hbm, wqkv_sc, C2, 3 * D),
        "sa": cols(wmod_hbm, wmod_sc, 0, D),
        "x1": rows(384, 512),
        "modB": cols(wmod_hbm, wmod_sc, 2 * D, 5 * D),
        "wo": (wo_hbm, wo_sc),
        "b1": (b1_hbm, b1_sc),
        "b2": (b2_hbm, b2_sc),
        "w1": (w1t_hbm, w1t_sc),
        "w2": (w2_hbm, w2_sc),
        "modC": cols(wmod_hbm, wmod_sc, 5 * D, 6 * D),
        "x2": rows(512, 640),
        "x3": rows(640, S),
    }
    copies = {name: pltpu.make_async_copy(src, dst, sems.at[n])
              for n, (name, (src, dst)) in enumerate(pairs.items())}

    def wait(*names):
        for name in names:
            copies[name].wait()

    def mod(n):
        return mod_sc[0:1, n * D:(n + 1) * D]

    def compute_mod(a, b):
        mod_sc[:, a:b] = jnp.dot(silu_sc[...], wmod_sc[:, a:b], preferred_element_type=F32)[0:8]

    def body(first):
        p_sc = p_sc0 if first else p_sc1
        p32 = p_sc.bitcast(U32)
        blk0 = 0 if first else NFIRST + (i - 1) * NSUB

        base = {scale: 0 if first else pl.multiple_of(blk0 * scale, scale) for scale in (64, 128)}

        def at(bb, scale, off=0):
            return base[scale] + (bb * scale + off)

        def rows_of(bb):
            return pl.ds(at(bb, 128), 128)

        lane = lax.broadcasted_iota(jnp.int32, (16, 128), 1)
        row = lax.broadcasted_iota(jnp.int32, (16, 128), 0)
        ql = lane & 31
        tri = [row <= ql, row + 16 <= ql]
        tri32 = (jnp.where(2 * row <= ql, jnp.uint32(0xFFFF), jnp.uint32(0))
                 | jnp.where(2 * row + 1 <= ql, jnp.uint32(0xFFFF0000), jnp.uint32(0)))
        bit0 = (lane & 32) == 0
        bit1 = lane < 64
        bit0_24 = (lax.broadcasted_iota(jnp.int32, (24, 128), 1) & 32) == 0
        sub8 = lax.broadcasted_iota(jnp.int32, (8, 128), 0) < 4
        z16 = jnp.zeros((16, 128), U32)
        always = lax.broadcasted_iota(jnp.int32, (8, 128), 1) >= z1
        qcode = ((lax.broadcasted_iota(jnp.int32, (40, 128), 1) >> 5)
                 ^ (lax.broadcasted_iota(jnp.int32, (40, 128), 0) // (DH // 2)))

        def chained(fn, x, nch):
            r = x.shape[0] // nch
            outs, zero = [], None
            for e in range(nch):
                if outs:
                    zero = jnp.where(always, 0.0, outs[-1][0:8, 0:128])
                outs.append(fn(x[r * e:r * e + r], zero))
            return jnp.concatenate(outs, axis=0)

        def ln1(rs, nch):
            return chained(lambda x, zero: _ln(x, zero) * (1.0 + mod(1)) + mod(0), x_sc[rs, :].astype(F32), nch)

        def pack(x, slot, r0=0):
            n = x.shape[0]
            p_sc[slot, r0:r0 + n, :] = x.astype(BF16)
            return p32[slot, r0 // 2:(r0 + n) // 2, :]

        def put_qkv(bb, qkv):
            qt = _xor_rows(qkv[:, 0:D] * QSCALE).T
            for t in range(5):
                q32[bb, 64 * t:64 * t + 64, :] = pack(qt[128 * t:128 * t + 128], t)
            full = jnp.concatenate([pack(qkv[:, D + 128 * t:D + 128 * t + 128], t, 128) for t in range(5)], axis=1)
            for g in range(NG):
                k32[g, pl.ds(at(bb, 64), 64), :] = full[:, _group_base(g):_group_base(g) + 128]
            vt = qkv[:, 2 * D:3 * D].T
            ones = jnp.ones((8, 128), F32)
            for hd in range(H):
                st = 8 * ((DH * hd) // 8)
                vt32[blk0 + bb, 16 * hd:16 * hd + 16, :] = pack(
                    jnp.concatenate([vt[st:st + 24], ones], axis=0), hd // 8, 32 * (hd % 8))

        hs, qkvs = {}, {}

        def qkv_stage(bb, lo, hi):
            if bb not in hs:
                hs[bb] = h_sc[...] if bb == 0 else ln1(rows_of(bb), 4).astype(BF16)
                qkvs[bb] = {}
            qkvs[bb][lo] = _dot_cols(hs[bb], wqkv_sc, lo, hi)
            if sum(v.shape[1] for v in qkvs[bb].values()) == 3 * D:
                put_qkv(bb, jnp.concatenate([qkvs[bb][k] for k in sorted(qkvs[bb])], axis=1))

        def sel(m, a, b):
            if a is None and b is None:
                return None
            return jnp.where(m, z16 if a is None else a, z16 if b is None else b)

        jobs = {}

        def stage_a(n, parts, g):
            off = 80 * g - _group_base(g)
            where, maxes = {}, {}
            used = [0] * 4
            for pi, (bb, cmin) in enumerate(parts):
                zq = q32[bb, 40 * g:40 * g + 40, :]
                for u in (range(4) if cmin == 0 else range(3, -1, -1)):
                    z8 = jnp.zeros((8, 128), U32)
                    qm = jnp.concatenate([z8] * (off // 16) + [jnp.where(qcode == u, zq, jnp.zeros_like(zq))]
                                         + [z8] * (3 - off // 16), axis=0)
                    kmin = max(1, cmin - u)

                    def keys(r, n_):
                        return k32[g, pl.ds(at(bb, 64, 16 * u - 128 + r), n_), :]

                    mid = [keys(16 * kmin, 128 - 16 * kmin)] if kmin < 8 else []
                    if cmin == 0:
                        kk = jnp.concatenate([keys(0, 8), keys(128, 8), keys(8, 8), keys(136, 8)] + mid, axis=0)
                        s = jnp.dot(_unpack(kk), _unpack(qm), preferred_element_type=F32)
                        sm = [jnp.where(tri[0], s[16:32], s[0:16]), jnp.where(tri[1], s[48:64], s[32:48]), s[64:]]
                    else:
                        kk = jnp.concatenate([keys(128, 16)] + mid, axis=0)
                        s = jnp.dot(_unpack(kk), _unpack(qm), preferred_element_type=F32)
                        sm = [jnp.where(tri[0], s[0:16], NEG), jnp.where(tri[1], s[16:32], NEG)]
                        sm += [s[32:]] if mid else []
                    sm = jnp.concatenate(sm, axis=0)
                    nr = sm.shape[0]
                    v = u if pi == 0 else 3 - u
                    buf = s_sc[(4 * n + v) % NP]
                    buf[z1, used[v]:used[v] + nr, :] = sm
                    for j, k in enumerate([0] + list(range(kmin, 8))):
                        where[pi, u, k] = (buf, used[v] + 32 * j)
                    used[v] += nr
                    acc = [sm[0:8], sm[8:16]]
                    for r in range(2, nr // 8):
                        acc[r % 2] = jnp.maximum(acc[r % 2], sm[8 * r:8 * r + 8])
                    maxes[pi, u] = jnp.max(jnp.maximum(acc[0], acc[1]), axis=0, keepdims=True)
            jobs[n] = (parts, g, where, maxes)

        def stage_b(n, prev=None):
            parts, g, where, maxes = jobs.pop(n)
            tiles = [(pi, t) for pi, (_, cmin) in enumerate(parts) for t in (1, 0, 2) if 4 * t >= cmin]
            if len(parts) == 2:
                tiles = tiles[::-1]
            items = []
            for pi, t in tiles:
                for c in (3, 2, 1, 0):
                    for u in range(4):
                        it = (pi, u, (4 * t + c - u) % 8)
                        if 0 <= 4 * t + c - u <= 8 and it not in items:
                            items.append(it)
            assert sorted(items) == sorted(where)
            ms = {k: jnp.broadcast_to(m, (8, 128)) for k, m in maxes.items()}
            pk = {}
            step = len(parts) + 1
            for e in range(0, len(items), step):
                for pi, u, k in items[e:e + step]:
                    buf, r0 = where[pi, u, k]
                    m = ms[pi, u] if prev is None else jnp.where(always, ms[pi, u], prev)
                    p = jnp.exp2(buf[z2, r0:r0 + 32, :] - jnp.concatenate([m] * 4, axis=0))
                    pk[pi, u, k] = pack(p, 4 * pi + u, 32 * k)
                    if (pi, u, k) == items[e]:
                        nxt = p[24:32]
                prev = nxt
            ph = {}
            for pi, (bb, cmin) in enumerate(parts):
                units = []
                for u in range(4):
                    if cmin == 0:
                        last = pk[pi, u, 0] & tri32
                        head = pk[pi, u, 0] ^ last
                    else:
                        last, head = pk[pi, u, 0], None
                    chunks = [head] + [pk.get((pi, u, k)) for k in range(1, 8)] + [last]
                    units.append([None] * u + chunks + [None] * (3 - u))
                for c in range(cmin, 12):
                    u0, u1, u2, u3 = (units[u][c] for u in range(4))
                    a0, a1, a2, a3 = sel(bit0, u0, u1), sel(bit0, u1, u0), sel(bit0, u2, u3), sel(bit0, u3, u2)
                    ph[pi, 0, c] = sel(bit1, a0, a2)
                    ph[pi, 1, c] = sel(bit1, a1, a3)
                    ph[pi, 2, c] = sel(bit1, a2, a0)
                    ph[pi, 3, c] = sel(bit1, a3, a1)
            part = {}
            for pi, t in tiles:
                for hh in range(4):
                    hd = 4 * g + hh
                    pt = jnp.concatenate([ph[pi, hh, c] for c in range(4 * t, 4 * t + 4)], axis=0)
                    part[pi, hh, t] = jnp.dot(_unpack(vt32[blk0 + parts[pi][0] - 2 + t, 16 * hd:16 * hd + 16, :]),
                                              _unpack(pt), preferred_element_type=F32)
            for pi, (bb, cmin) in enumerate(parts):
                outs = []
                for hh in range(4):
                    ds = [part[pi, hh, t] for pj, t in tiles if pj == pi]
                    o = functools.reduce(jnp.add, [d[0:24] for d in ds])
                    den = functools.reduce(jnp.add, [d[24:32] for d in ds])
                    r = pl.reciprocal(den, approx=True)
                    r = r * (2.0 - den * r)
                    o = o * jnp.concatenate([r, r, r], axis=0)
                    if hh == 1:
                        o = jnp.where(bit0_24, pltpu.roll(o, 96, 1), pltpu.roll(o, 32, 1))
                    elif hh == 2:
                        o = pltpu.roll(o, 64, 1)
                    elif hh == 3:
                        o = jnp.where(bit0_24, pltpu.roll(o, 32, 1), pltpu.roll(o, 96, 1))
                    outs.append(o)
                for e in range(2):
                    oa, ob = outs[2 * e], outs[2 * e + 1]
                    pair = jnp.concatenate([oa[0:16], jnp.where(sub8, oa[16:24], ob[0:8]), ob[8:24]], axis=0)
                    ot_sc[bb][z1, 80 * g + 40 * e:80 * g + 40 * e + 40, :] = pair

        def attention(*plist, before=None, after=None, dep=None):
            todo = [(parts, g) for parts in plist for g in range(NG)]
            stage_a(0, *todo[0])
            for n in range(len(todo) - 1):
                stage_a(n + 1, *todo[n + 1])
                if before and n in before:
                    before[n]()
                stage_b(n, dep if n == 0 else None)
                if after and n in after:
                    after[n]()
            return functools.partial(stage_b, len(todo) - 1)

        x1s, ys, gs = {}, {}, {}

        def wo_stage(bb, halves=False, nch=1, between=None):
            o = ot_sc[bb][z2].T
            if between is not None:
                attn = [_dot_cols(o, wo_sc, 0, 512)]
                between()
                attn = jnp.concatenate(attn + [_dot_cols(o, wo_sc, 512, D, 4)], axis=1)
            elif halves:
                attn = jnp.concatenate([_dot_cols(o[64 * e:64 * e + 64], wo_sc, 0, D, 2) for e in range(2)], axis=0)
            else:
                attn = _dot_cols(o, wo_sc, 0, D, 4)
            x1s[bb] = x_sc[rows_of(bb), :].astype(F32) + mod(2) * attn
            ys[bb] = chained(lambda x, zero: _ln(_ln(x, zero) * (1.0 + mod(4)) + mod(3)), x1s[bb], nch)

        def w1_stage(bb, between=None, after=None):
            y = ys[bb]
            if between is None:
                head = _dot_cols(y, w1t_sc, 0, 768, nt=True)
            else:
                head = _dot_cols(y, w1t_sc, 0, 512, nt=True)
                between()
                head = jnp.concatenate([head, _dot_cols(y, w1t_sc, 512, 768, nt=True)], axis=1)
            fm = F - 64
            tail = (lax.dot_general(w1t_sc[fm:F, 0:512], y[:, 0:512].astype(BF16), NT, preferred_element_type=F32).T
                    + lax.dot_general(y[:, 512:D].astype(BF16), w1t_sc[fm:F, 512:D], NT, preferred_element_type=F32))
            h1 = jnp.concatenate([head, _dot_cols(y, w1t_sc, 768, fm, nt=True), tail], axis=1)
            h1 = h1 + b1_sc[...].astype(F32).reshape(1, F)
            if after is None:
                gs[bb] = _gelu(h1)
            else:
                g = [_gelu(h1[:, 0:fm - 256]), None, _gelu(h1[:, fm:F])]
                after()
                g[1] = _gelu(h1[:, fm - 256:fm])
                gs[bb] = jnp.concatenate(g, axis=1)

        def w2_stage(bb, lo=0, hi=D, parts=1, with_mod=False):
            b2 = b2_sc[...].astype(F32).reshape(1, D)
            mlp = _dot_cols(gs[bb], w2_sc, lo, hi, parts) + b2[:, lo:hi]
            if with_mod:
                compute_mod(5 * D + lo, 5 * D + hi)
            gb = mod_sc[0:1, 5 * D + lo:5 * D + hi]
            o_sc[rows_of(bb), lo:hi] = (x1s[bb][:, lo:hi] + gb * mlp).astype(o_sc.dtype)

        def flush(bb, lo=0, hi=D):
            pltpu.make_async_copy(o_sc.at[rows_of(bb), lo:hi], o_hbm.at[rows_of(bb), lo:hi], osem).start()

        if first:
            for cp in copies.values():
                cp.start()
            wait("c", "x0")
            c = c_sc[...].astype(F32)
            silu_sc[...] = jnp.broadcast_to(c * jax.nn.sigmoid(c), (16, D)).astype(BF16)
            xn = _ln(x_sc[0:384, :].astype(F32))
            wait("ca")
            compute_mod(D, 2 * D)
            t = [xn[128 * bb:128 * bb + 128] * (1.0 + mod(1)) for bb in range(3)]
            res = [[], [], []]
            wait("wa")
            for bb in range(3):
                res[bb].append(_dot_cols(t[bb], wqkv_sc, 0, C1, 4 if bb == 2 else 1))
            wait("wb")
            for bb in range(3):
                res[bb].append(_dot_cols(t[bb], wqkv_sc, C1, C2, 4 if bb == 2 else 1))
            wait("wc")
            for bb in range(2):
                res[bb].append(_dot_cols(t[bb], wqkv_sc, C2, 3 * D, 2 if bb == 1 else 1))
            wait("sa", "x1")
            for c0 in range(0, D, 128):
                res[2].append(_dot_cols(t[2], wqkv_sc, C2 + c0, C2 + c0 + 128))
                compute_mod(c0, c0 + 128)
            res[2].append(_dot_cols(t[2], wqkv_sc, C2 + D, 3 * D))
            h3 = ln1(rows_of(3), 1)
            sa = jnp.broadcast_to(mod(0), (16, D))
            r3 = jnp.concatenate(
                [_dot_cols(jnp.concatenate([h3, sa], axis=0), wqkv_sc, 0, QE),
                 jnp.concatenate([_dot_cols(h3, wqkv_sc, QE, 3 * D, 4), _dot_cols(sa, wqkv_sc, QE, 3 * D)], axis=0)],
                axis=1)
            for bb in range(4):
                put_qkv(bb, r3[0:128] if bb == 3 else jnp.concatenate(res[bb], axis=1) + r3[128:129])

            low = []

            def mid_weights():
                wait("modB", "wo", "b1", "b2", "w1")
                low.append(jnp.dot(silu_sc[:, 512:D], wmod_sc[512:D, 2 * D:5 * D], preferred_element_type=F32)[0:8])

            def mod_piece(c0, c1):
                top = jnp.dot(silu_sc[:, 0:512], wmod_sc[0:512, 2 * D + c0:2 * D + c1], preferred_element_type=F32)
                mod_sc[:, 2 * D + c0:2 * D + c1] = top[0:8] + low[0][:, c0:c1]

            pieces = {2 * NG - 1 + j: functools.partial(mod_piece, c0, min(c0 + 256, 3 * D))
                      for j, c0 in enumerate(range(0, 3 * D, 256))}
            fin = attention([(1, 4), (0, 8)], [(2, 0)], [(3, 0)], before={2 * NG - 2: mid_weights}, after=pieces)
            wo_stage(0, between=fin)
            wo_stage(1)
            wo_stage(2, nch=4)
            w1_stage(0)
            w1_stage(1, after=functools.partial(wait, "w2", "modC", "x2"))
            for c0 in range(0, D, 128):
                w2_stage(0, c0, c0 + 128, with_mod=True)
                if c0 == 0:
                    wo_stage(3, halves=True)
            flush(0)
            w1_stage(2)
            w2_stage(1)
            flush(1)
            w1_stage(3)
            w2_stage(2)
            flush(2)
            h_sc[...] = ln1(rows_of(NFIRST), 8).astype(BF16)
            w2_stage(3, parts=2)
            flush(3)
        else:
            qkv_stage(0, 0, 3 * D)
            qkv_stage(1, QE, 3 * D)
            fin = attention([(0, 0)])
            qkv_stage(1, 0, 512)
            fin()
            qkv_stage(1, 512, 2 * D)
            wo_stage(0)
            qkv_stage(1, 2 * D, QE)
            y0 = functools.reduce(jnp.maximum, [ys[0][8 * r:8 * r + 8, 0:128] for r in range(16)])
            fin = attention([(1, 0)], dep=y0)
            w1_stage(0, fin)
            wo_stage(1, nch=4)
            w2_stage(0)
            w1_stage(1)
            flush(0)
            nxt = pl.multiple_of(jnp.minimum(blk0 + NSUB, S // 128 - 1) * 128, 128)
            h_sc[...] = ln1(pl.ds(nxt, 128), 8).astype(BF16)
            w2_stage(1, 0, 512)
            flush(1, 0, 512)
            w2_stage(1, 512, D, 2)
            flush(1, 512, D)

    pl.when(i == 1)(functools.partial(wait, "x3"))
    pl.when(i == 0)(functools.partial(body, True))
    pl.when(i > 0)(functools.partial(body, False))

    @pl.when(i == NSTEP - 1)
    def _():
        pltpu.make_async_copy(o_sc, o_hbm, osem).wait()


@jax.jit
def pallas_adaLN_cond__sliding_block__mixer_channel_mlp__prompt_kernel(
    A_x, A_wqkv, A_wo, B_x, B_w1, B_b1, B_w2, B_b2, c, w_mod):
    del B_x
    out = pl.pallas_call(
        _kernel,
        grid=(NSTEP,),
        in_specs=[pl.BlockSpec(memory_space=pl.ANY)] * 9,
        out_specs=pl.BlockSpec(memory_space=pl.ANY),
        out_shape=jax.ShapeDtypeStruct((S, D), A_x.dtype),
        scratch_shapes=[
            pltpu.SemaphoreType.DMA((17,)),
            pltpu.SemaphoreType.DMA(()),
            pltpu.VMEM((S, D), BF16),
            pltpu.VMEM((D, 3 * D), BF16),
            pltpu.VMEM((D, D), BF16),
            pltpu.VMEM((F, D), BF16),
            pltpu.VMEM((F, D), BF16),
            pltpu.VMEM((D, 6 * D), BF16),
            pltpu.VMEM((S, D), BF16),
            pltpu.VMEM((128, D), BF16),
            pltpu.VMEM((NFIRST, D // 2, 128), U32),
            pltpu.VMEM((NG, S // 2, 128), U32),
            pltpu.VMEM((S // 128, H * 16, 128), U32),
            pltpu.VMEM((8, 256, 128), BF16),
            pltpu.VMEM((8, 256, 128), BF16),
            pltpu.VMEM((8, 4096), F32),
        ] + [pltpu.VMEM((1, D, 128), F32)] * NFIRST
          + [pltpu.VMEM((1, 288, 128), F32)] * NP
          + [pltpu.VMEM((16, D), BF16),
             pltpu.VMEM((F,), BF16),
             pltpu.VMEM((D,), BF16),
             pltpu.VMEM((1, D), BF16)],
        compiler_params=pltpu.CompilerParams(
            dimension_semantics=("arbitrary",), vmem_limit_bytes=100 * 1024 * 1024,
            disable_bounds_checks=True, disable_semaphore_checks=True),
        name="fused_block",
    )(A_x.reshape(S, D), A_wqkv, A_wo, B_w1.T, B_b1, B_w2, B_b2, c, w_mod)
    return out.reshape(1, S, D)
```
